```python
import jax
import jax.numpy as jnp

def _softmax(x, axis=-1):
    return jax.nn.softmax(x, axis=axis)

def _gelu(x):
    return jax.nn.gelu(x, approximate=True)

def _silu(x):
    return jax.nn.silu(x)

def _sigmoid(x):
    return jax.nn.sigmoid(x)

def _layernorm(x, axis=-1, eps=1e-05):
    m = jnp.mean(x, axis=axis, keepdims=True)
    v = jnp.var(x, axis=axis, keepdims=True)
    return (x - m) / jnp.sqrt(v + eps)

def _scatter_add(tgt, idx, src, axis=0):
    return tgt.at[idx].add(src)

def _segment_sum(src, seg, n):
    return jax.ops.segment_sum(src, seg, n)

class _Rng:

    def __init__(self, key):
        self._k = key

    def _next(self):
        self._k, sub = jax.random.split(self._k)
        return sub

    def normal(self, shape):
        return jax.random.normal(self._next(), shape, dtype=jnp.bfloat16)

    def randint(self, lo, hi, shape):
        return jax.random.randint(self._next(), shape, lo, hi, dtype=jnp.int32)

    def uniform(self, shape, lo=0.0, hi=1.0):
        return jax.random.uniform(self._next(), shape, jnp.bfloat16, lo, hi)

    def permutation(self, n):
        return jax.random.permutation(self._next(), n)
kernel_name = 'parallel_sum__memory_aug_recurrent_mem_tr__moe_arch_mod__prompt'

def setup_inputs():
    _rng = _Rng(jax.random.key(int.from_bytes(__import__("os").urandom(4), "little")))
    _w = lambda a: (lambda t: t.astype(jnp.bfloat16) if jnp.issubdtype(t.dtype, jnp.floating) else t)(jnp.asarray(a))

    def _A_setup():
        B, S, Dm = (1, 2048, 1024)
        H, Dh = (32, 128)
        M, seg = (8, 32)
        seg = min(seg, S)
        S = S // seg * seg
        return {'x': _w((lambda *s: _rng.normal(s) * 0.05)(B, S, Dm)), 'mem0': _w((lambda *s: _rng.normal(s) * 0.05)(B, M, Dm)), 'Wq': _w((lambda *s: _rng.normal(s) * 0.05)(Dm, H, Dh) * Dm ** (-0.5)), 'Wk': _w((lambda *s: _rng.normal(s) * 0.05)(Dm, H, Dh) * Dm ** (-0.5)), 'Wv': _w((lambda *s: _rng.normal(s) * 0.05)(Dm, H, Dh) * Dm ** (-0.5)), 'Wo': _w((lambda *s: _rng.normal(s) * 0.05)(H, Dh, Dm) * (H * Dh) ** (-0.5)), 'seg_len': seg}
    _A_in = _A_setup()

    def _B_setup():
        B, S, D, F, C = (1, 2048, 1024, 3584, 2)
        return {'x': _w((lambda *s: _rng.normal(s) * 0.05)(B, S, D)), 'w_r': _w((lambda *s: _rng.normal(s) * 0.05)(D)), 'w_gate': _w((lambda *s: _rng.normal(s) * 0.05)(D, F)), 'w_up': _w((lambda *s: _rng.normal(s) * 0.05)(D, F)), 'w_down': _w((lambda *s: _rng.normal(s) * 0.05)(F, D))}
    _B_in = _B_setup()
    return {'A_x': _A_in['x'], 'A_mem0': _A_in['mem0'], 'A_Wq': _A_in['Wq'], 'A_Wk': _A_in['Wk'], 'A_Wv': _A_in['Wv'], 'A_Wo': _A_in['Wo'], 'A_seg_len': _A_in['seg_len'], 'B_x': _B_in['x'], 'B_w_r': _B_in['w_r'], 'B_w_gate': _B_in['w_gate'], 'B_w_up': _B_in['w_up'], 'B_w_down': _B_in['w_down']}

def reference(A_x, A_mem0, A_Wq, A_Wk, A_Wv, A_Wo, A_seg_len, B_x, B_w_r, B_w_gate, B_w_up, B_w_down):

    def _A_ref(x, mem0, Wq, Wk, Wv, Wo, seg_len):
        B, S, Dm = x.shape
        H, Dh = (Wq.shape[1], Wq.shape[2])
        M = mem0.shape[1]
        scale = Dh ** (-0.5)
        n_seg = S // seg_len
        L = M + seg_len
        idx = jnp.arange(L)
        mask = (idx[:, None] < M) | (idx[:, None] >= idx[None, :])
        mem = mem0
        outs = []
        for s in range(n_seg):
            xs = x[:, s * seg_len:(s + 1) * seg_len, :].copy()
            h = jnp.concatenate([mem, xs], axis=1)
            q = jnp.einsum('btd,dhe->bhte', h, Wq)
            k = jnp.einsum('btd,dhe->bhte', h, Wk)
            v = jnp.einsum('btd,dhe->bhte', h, Wv)
            scores = jnp.einsum('bhqe,bhke->bhqk', q, k) * scale
            scores = jnp.where(mask[None, None], scores, -1000000000.0)
            p = _softmax(scores, axis=-1)
            o = jnp.einsum('bhqk,bhke->bhqe', p, v)
            o = jnp.einsum('bhte,hed->btd', o, Wo)
            mem = o[:, :M, :].copy()
            outs.append(o[:, M:, :])
        return jnp.concatenate(outs, axis=1)

    def _B_ref(x, w_r, w_gate, w_up, w_down):
        B, S, D = x.shape
        C = 2
        r = x @ w_r
        idx = jnp.argsort(-r, axis=-1)[:, :C]
        idx_e = jnp.repeat(idx.reshape(B, C, 1), D, axis=2)
        x_sel = jnp.take_along_axis(x, idx_e, axis=1)
        g = _silu(x_sel @ w_gate)
        u = x_sel @ w_up
        y = g * u @ w_down
        r_sel = _sigmoid(jnp.take_along_axis(r, idx, axis=1))
        y = y * r_sel.reshape(B, C, 1)
        b_off = (jnp.arange(B) * S).reshape(B, 1)
        flat_idx = (idx + b_off).reshape(B * C)
        zero = (x * 0.0).reshape(B * S, D)
        upd = _scatter_add(zero, flat_idx, y.reshape(B * C, D), axis=0)
        return x + upd.reshape(B, S, D)
    x = A_x
    xn = _layernorm(x, axis=-1)
    return x + _A_ref(xn, A_mem0, A_Wq, A_Wk, A_Wv, A_Wo, A_seg_len) + _B_ref(xn, B_w_r, B_w_gate, B_w_up, B_w_down)
```

```python
import functools

import jax
import jax.numpy as jnp
import numpy as np
from jax import lax
import jax.experimental.pallas as pl
import jax.experimental.pallas.tpu as pltpu

F32 = jnp.float32
BF16 = jnp.bfloat16
U32 = jnp.uint32
LANES = 128
RAW_SLOTS = 4
NEG = -1000000000.0


def _rnd(v):
    return v.astype(BF16).astype(F32)


def _layernorm(x):
    mean = jnp.mean(x, axis=-1, keepdims=True)
    xc = x - mean
    var = jnp.mean(xc * xc, axis=-1, keepdims=True)
    sd = _rnd(jnp.sqrt(_rnd(_rnd(var) + np.float32(np.asarray(1e-5, BF16)))))
    return _rnd(_rnd(x - _rnd(mean)) / sd)


def _kernel(x_hbm, mem0_ref, wq_hbm, wk_hbm, wv_hbm, wo_hbm, wr_ref, wg_hbm, wu_hbm, wd_hbm,
            out_hbm,
            xraw, xn, xa, base, raw, wqkv, wo, sq, so, wg, wu, wd, fill_ref,
            sem_x, sem_raw, sem_wo, sem_b, sem_out, *, cfg):
    n_seg, seg, D = xraw.shape
    M = mem0_ref.shape[1]
    n_pair = wqkv.shape[0]
    KT = D // LANES
    FT = wg.shape[0]
    R = 2 * (seg + M)
    scale = float(LANES) ** -0.5

    w_u32 = [w.bitcast(U32) for w in (wq_hbm, wk_hbm, wv_hbm)]

    def raw_copy(g, slot, c):
        return pltpu.make_async_copy(w_u32[c].at[:, g, :], raw.at[slot, c], sem_raw.at[slot, c])

    x0_copy = pltpu.make_async_copy(x_hbm.at[:, pl.ds(0, M), :], xraw.at[:, pl.ds(0, M), :], sem_x.at[0])
    x1_copy = pltpu.make_async_copy(
        x_hbm.at[:, pl.ds(M, seg - M), :], xraw.at[:, pl.ds(M, seg - M), :], sem_x.at[1])

    def wo_copy(j):
        return pltpu.make_async_copy(wo_hbm.at[:, pl.ds(j * LANES, LANES)], wo.at[j], sem_wo.at[0])

    def b_copies():
        cps = []
        for j in range(FT):
            cps.append(pltpu.make_async_copy(wg_hbm.at[:, pl.ds(j * LANES, LANES)], wg.at[j], sem_b.at[0]))
            cps.append(pltpu.make_async_copy(wu_hbm.at[:, pl.ds(j * LANES, LANES)], wu.at[j], sem_b.at[1]))
        for j in range(KT):
            cps.append(pltpu.make_async_copy(wd_hbm.at[:, pl.ds(j * LANES, LANES)], wd.at[j], sem_b.at[2]))
        return cps

    x0_copy.start()
    for g in range(RAW_SLOTS):
        for c in range(3):
            raw_copy(g, g, c).start()
        if g == 0:
            x1_copy.start()

    w_r = wr_ref[...].astype(F32)
    lane8 = lax.broadcasted_iota(jnp.int32, (M, LANES), 1)

    def router(racc, xn_rows, grp):
        r = _rnd(jnp.sum(xn_rows * w_r, axis=-1, keepdims=True))
        return tuple(jnp.where(lane8 + LANES * i == grp, r, a) for i, a in enumerate(racc))

    def unzip(g, slot):
        for c in range(3):
            w = raw[slot, c]
            wqkv[g, 2 * c] = pltpu.bitcast(w << 16, F32).astype(BF16)
            wqkv[g, 2 * c + 1] = pltpu.bitcast(w & np.uint32(0xFFFF0000), F32).astype(BF16)

    def w_pair(g):
        return jnp.concatenate([wqkv[g, j] for j in range(6)], axis=1)

    def head_and_pos(i):
        head = jnp.where(i < 2 * seg, i // seg, (i - 2 * seg) // M)
        j = i % seg
        pos = jnp.where(i < 2 * seg, jnp.where(j < M, j, j + M), i % M + M)
        return head, pos

    qh, qp = head_and_pos(lax.broadcasted_iota(jnp.int32, (R, R), 0))
    kh, kp = head_and_pos(lax.broadcasted_iota(jnp.int32, (R, R), 1))
    visible = (qp < M) | (qp >= kp)
    fill_ref[...] = jnp.where(qh == kh, jnp.where(visible, 0.0, NEG), -jnp.inf).astype(F32)

    x0_copy.wait()

    def ln0_body(i, racc):
        for u in range(2):
            s = 4 * i + 2 * u
            xs = jnp.concatenate([xraw[s, 0:M, :].astype(F32), xraw[s + 1, 0:M, :].astype(F32)], axis=0)
            y = _layernorm(xs)
            yb = y.astype(BF16)
            for k in range(KT):
                xa[k, pl.ds(pl.multiple_of(s * M, 2 * M), 2 * M), :] = yb[:, k * LANES:(k + 1) * LANES]
            for t in range(2):
                xn[s + t, 0:M, :] = y[t * M:(t + 1) * M].astype(BF16)
                base[s + t, 0:M, :] = xs[t * M:(t + 1) * M] + y[t * M:(t + 1) * M]
                racc = router(racc, y[t * M:(t + 1) * M], (s + t) * (seg // M))
        return racc

    n_r = n_seg * (seg // M) // LANES
    racc = lax.fori_loop(0, n_seg // 4, ln0_body, tuple(jnp.zeros((M, LANES), F32) for _ in range(n_r)))

    for c in range(3):
        raw_copy(0, 0, c).wait()
    unzip(0, 0)
    for c in range(3):
        raw_copy(RAW_SLOTS, 0, c).start()
    x1_copy.wait()

    segs_per = n_seg // n_pair

    def phase_a(g, racc):
        nxt = jnp.minimum(g + 1, n_pair - 1)
        slot = nxt % RAW_SLOTS

        @pl.when(g + 1 < n_pair)
        def _():
            for c in range(3):
                raw_copy(nxt, slot, c).wait()

        lhs = jnp.concatenate([xa[k] for k in range(KT)], axis=1)
        for c in range(3):
            w = jnp.concatenate([wqkv[g, 2 * c], wqkv[g, 2 * c + 1]], axis=1)
            res = jnp.dot(lhs, w, preferred_element_type=F32)
            a = res[:, :LANES].reshape(n_seg, M, LANES)
            b = res[:, LANES:].reshape(n_seg, M, LANES)
            sq[g, c] = jnp.concatenate([a, b], axis=1).astype(BF16)

        unzip(nxt, slot)

        for t in range(segs_per):
            s = g * segs_per + t
            xs = xraw[s, M:seg, :].astype(F32)
            y = _layernorm(xs)
            xn[s, M:seg, :] = y.astype(BF16)
            base[s, M:seg, :] = xs + y
            for u in range(1, seg // M):
                racc = router(racc, y[(u - 1) * M:u * M], s * (seg // M) + u)

        @pl.when(g + 1 + RAW_SLOTS < n_pair)
        def _():
            for c in range(3):
                raw_copy(g + 1 + RAW_SLOTS, slot, c).start()

        @pl.when(g + 1 + RAW_SLOTS == n_pair)
        def _():
            for j in range(KT):
                wo_copy(j).start()
            for cp in b_copies():
                cp.start()

        return racc

    racc = lax.fori_loop(0, n_pair, phase_a, racc)
    for j in range(KT):
        wo_copy(j).wait()

    def step(s, mem):
        xs = xn[s]
        top = jnp.concatenate([mem, xs[0:2 * M].astype(F32)[M:]], axis=0).astype(BF16)
        h = jnp.concatenate([top, xs[2 * M:]], axis=0)
        qkv, probs, outs = {}, {}, {}

        def proj(g):
            res = jnp.dot(h, w_pair(g), preferred_element_type=F32).astype(BF16)
            qkv[g] = [
                jnp.concatenate([res[:, (2 * c) * LANES:(2 * c + 1) * LANES],
                                 res[:, (2 * c + 1) * LANES:(2 * c + 2) * LANES],
                                 sq[g, c, s]], axis=0)
                for c in range(3)]

        def qk(g):
            q, k, v = qkv.pop(g)
            sc = lax.dot_general(q, k, (((1,), (1,)), ((), ())), preferred_element_type=F32) * scale
            fill = fill_ref[...]
            sc = jnp.where(fill == 0.0, sc, fill)
            e = jnp.exp(sc - jnp.max(sc, axis=-1, keepdims=True))
            probs[g] = (e.astype(BF16), 1.0 / jnp.sum(e, axis=-1, keepdims=True), v)

        def pv(g):
            e, inv, v = probs.pop(g)
            o = jnp.dot(e, v, preferred_element_type=F32) * inv
            so[2 * g, s] = o[2 * seg:2 * seg + M]
            so[2 * g + 1, s] = o[2 * seg + M:]
            ob = o[:2 * seg].astype(BF16)
            outs[g] = jnp.concatenate([ob[:seg], ob[seg:]], axis=1)

        def oproj(g0, g1, acc):
            lhs = jnp.concatenate([outs.pop(g) for g in range(g0, g1)], axis=1)
            w = jnp.concatenate([wo[j, 2 * g0 * LANES:2 * g1 * LANES, :] for j in range(KT)], axis=1)
            res = jnp.dot(lhs, w, preferred_element_type=F32)
            return res if acc is None else acc + res

        acc = None
        for op in cfg["order"]:
            if op[0] == "proj":
                proj(op[1])
            elif op[0] == "qk":
                qk(op[1])
            elif op[0] == "pv":
                pv(op[1])
            else:
                acc = oproj(op[1], op[2], acc)
        base[s, M:seg, :] = base[s, M:seg, :] + acc[M:]
        return acc[:M]

    lax.fori_loop(0, n_seg, step, mem0_ref[0].astype(F32))

    tok = [lax.broadcasted_iota(jnp.int32, (M, LANES), 0) + M * (lane8 + LANES * i) for i in range(n_r)]
    keys = [jnp.where(a != a, -jnp.inf, a) for a in racc]
    big = np.int32(n_seg * seg)

    def pick(keys, cand):
        best = jnp.max(functools.reduce(jnp.maximum, [jnp.where(c, k, -jnp.inf) for k, c in zip(keys, cand)]))
        return jnp.min(functools.reduce(
            jnp.minimum, [jnp.where(c & (k == best), t, big) for k, t, c in zip(keys, tok, cand)]))

    i0 = pick(keys, [t >= 0 for t in tok])
    i1 = pick(keys, [t != i0 for t in tok])
    row = lax.broadcasted_iota(jnp.int32, (seg, D), 0)
    row16 = lax.broadcasted_iota(jnp.int32, (2 * M, D), 0)
    x_sel = jnp.zeros((2 * M, D), F32)
    for n, i in enumerate((i0, i1)):
        blk = xn[i // seg].astype(F32)
        x_sel = jnp.where(row16 == n, jnp.sum(jnp.where(row == i % seg, blk, 0.0), axis=0, keepdims=True), x_sel)
    gate_r = jax.nn.sigmoid(_rnd(jnp.sum(x_sel * w_r, axis=-1, keepdims=True)))
    x_sel = x_sel.astype(BF16)
    for cp in b_copies():
        cp.wait()
    gt = jnp.dot(x_sel, jnp.concatenate([wg[j] for j in range(FT)], axis=1), preferred_element_type=F32)
    up = jnp.dot(x_sel, jnp.concatenate([wu[j] for j in range(FT)], axis=1), preferred_element_type=F32)
    hid = (gt * jax.nn.sigmoid(gt) * up).astype(BF16)
    y = jnp.dot(hid, jnp.concatenate([wd[j] for j in range(KT)], axis=1), preferred_element_type=F32) * gate_r
    for n, i in enumerate((i0, i1)):
        base[i // seg] = base[i // seg] + jnp.where(row == i % seg, y[n:n + 1], 0.0)

    cs = cfg["c_segs"]
    n_chunk = n_seg // cs

    def out_copy(c):
        return pltpu.make_async_copy(xraw.at[pl.ds(c * cs, cs)], out_hbm.at[pl.ds(c * cs, cs)], sem_out.at[c])

    def phase_c(c, carry):
        s0 = c * cs
        lhs = jnp.concatenate(
            [so[hd, pl.ds(s0, cs)].reshape(cs * M, LANES).astype(BF16) for hd in range(2 * n_pair)], axis=1)
        w = jnp.concatenate([wo[j] for j in range(KT)], axis=1)
        res = jnp.dot(lhs, w, preferred_element_type=F32).reshape(cs, M, D)
        b = base[pl.ds(s0, cs)]
        xraw[pl.ds(s0, cs)] = jnp.concatenate([b[:, :M] + res, b[:, M:]], axis=1).astype(BF16)
        out_copy(c).start()
        return carry

    lax.fori_loop(0, n_chunk, phase_c, 0)
    for c in range(n_chunk):
        out_copy(c).wait()


def _order(n_pair=16, lag_qk=1, lag_pv=2, cuts=(8, 14, 16)):
    ops = []
    tail = [("oproj", a, b) for a, b in zip((0,) + tuple(cuts[:-1]), cuts)]
    for t in range(n_pair + lag_pv):
        if t < n_pair:
            ops.append(("proj", t))
        elif tail:
            ops.append(tail.pop(0))
        if 0 <= t - lag_pv < n_pair:
            ops.append(("pv", t - lag_pv))
        if 0 <= t - lag_qk < n_pair:
            ops.append(("qk", t - lag_qk))
    return tuple(ops + tail)


DEFAULT_CFG = dict(order=_order(), c_segs=16)


def make(cfg=None):
    cfg = dict(DEFAULT_CFG, **(cfg or {}))

    @functools.partial(jax.jit, static_argnames=["A_seg_len"])
    def fn(A_x, A_mem0, A_Wq, A_Wk, A_Wv, A_Wo, A_seg_len, B_x, B_w_r, B_w_gate, B_w_up, B_w_down):
        del B_x
        B, S, D = A_x.shape
        _, H, E = A_Wq.shape
        M = A_mem0.shape[1]
        F = B_w_gate.shape[1]
        seg = A_seg_len
        n_seg = S // seg
        n_pair = H // 2
        KT, FT = D // LANES, F // LANES
        R = 2 * (seg + M)
        hbm = pl.BlockSpec(memory_space=pl.ANY)
        vmem = pl.BlockSpec(memory_space=pltpu.VMEM)
        out = pl.pallas_call(
            functools.partial(_kernel, cfg=cfg),
            out_shape=jax.ShapeDtypeStruct((n_seg, seg, D), BF16),
            in_specs=[hbm, vmem, hbm, hbm, hbm, hbm, vmem, hbm, hbm, hbm],
            out_specs=hbm,
            scratch_shapes=[
                pltpu.VMEM((n_seg, seg, D), BF16),
                pltpu.VMEM((n_seg, seg, D), BF16),
                pltpu.VMEM((KT, n_seg * M, LANES), BF16),
                pltpu.VMEM((n_seg, seg, D), F32),
                pltpu.VMEM((RAW_SLOTS, 3, D, LANES), U32),
                pltpu.VMEM((n_pair, 6, D, LANES), BF16),
                pltpu.VMEM((KT, H * E, LANES), BF16),
                pltpu.VMEM((n_pair, 3, n_seg, 2 * M, LANES), BF16),
                pltpu.VMEM((H, n_seg, M, LANES), F32),
                pltpu.VMEM((FT, D, LANES), BF16),
                pltpu.VMEM((FT, D, LANES), BF16),
                pltpu.VMEM((KT, F, LANES), BF16),
                pltpu.VMEM((R, R), F32),
                pltpu.SemaphoreType.DMA((2,)),
                pltpu.SemaphoreType.DMA((RAW_SLOTS, 3)),
                pltpu.SemaphoreType.DMA((1,)),
                pltpu.SemaphoreType.DMA((3,)),
                pltpu.SemaphoreType.DMA((n_seg // cfg["c_segs"],)),
            ],
            compiler_params=pltpu.CompilerParams(
                vmem_limit_bytes=120 * 1024 * 1024, flags=cfg.get("flags")),
        )(A_x.reshape(n_seg, seg, D), A_mem0, A_Wq, A_Wk, A_Wv, A_Wo.reshape(H * E, D),
          B_w_r.reshape(1, D), B_w_gate, B_w_up, B_w_down)
        return out.reshape(B, S, D)

    return fn


pallas_parallel_sum__memory_aug_recurrent_mem_tr__moe_arch_mod__prompt_kernel = make()
```

```python
import functools

import jax
import jax.numpy as jnp
import numpy as np
from jax import lax
import jax.experimental.pallas as pl
import jax.experimental.pallas.tpu as pltpu

F32 = jnp.float32
BF16 = jnp.bfloat16
U32 = jnp.uint32
LANES = 128
NEG = -1000000000.0


def _rnd(v):
    return v.astype(BF16).astype(F32)


def _b16(u):
    return pltpu.bitcast(u, BF16)


def _layernorm(x):
    mean = jnp.mean(x, axis=-1, keepdims=True)
    xc = x - mean
    var = jnp.mean(xc * xc, axis=-1, keepdims=True)
    sd = _rnd(jnp.sqrt(_rnd(_rnd(var) + np.float32(np.asarray(1e-5, BF16)))))
    return _rnd(_rnd(x - _rnd(mean)) / sd)


def _kernel(x_hbm, mem0_ref, wq_hbm, wk_hbm, wv_hbm, wo_hbm, wr_ref, wg_hbm, wu_hbm, wd_hbm,
            out_hbm,
            xraw, xn, xa, base, raw, wqkv, wo, sq, so, wg, wu, wd, fill_ref,
            sem_x0, sem_x1, sem_raw, sem_wo, sem_b, sem_out, *, cfg):
    n_seg, seg, D = xraw.shape
    M = mem0_ref.shape[1]
    n_pair = wqkv.shape[0]
    slots = raw.shape[0]
    KT = D // LANES
    FT = wg.shape[0]
    R = 2 * (seg + M)
    scale = float(LANES) ** -0.5
    segs_per = n_seg // n_pair
    n_x0 = sem_x0.shape[0]

    w_u32 = [w.bitcast(U32) for w in (wq_hbm, wk_hbm, wv_hbm)]

    def raw_copy(g, slot, c):
        return pltpu.make_async_copy(w_u32[c].at[:, g, :], raw.at[slot, c], sem_raw.at[slot, c])

    def x0_copy(i):
        ss = pl.ds(i * (n_seg // n_x0), n_seg // n_x0)
        return pltpu.make_async_copy(x_hbm.at[ss, pl.ds(0, M), :], xraw.at[ss, pl.ds(0, M), :], sem_x0.at[i])

    def x1_copy(g):
        ss = pl.ds(g * segs_per, segs_per)
        return pltpu.make_async_copy(
            x_hbm.at[ss, pl.ds(M, seg - M), :], xraw.at[ss, pl.ds(M, seg - M), :], sem_x1.at[g])

    def wo_copy(j):
        return pltpu.make_async_copy(
            wo_hbm.at[:, pl.ds(pl.multiple_of(j * LANES, LANES), LANES)], wo.at[j], sem_wo.at[0])

    def b_copies():
        cps = []
        for j in range(FT):
            cps.append(pltpu.make_async_copy(wg_hbm.at[:, pl.ds(j * LANES, LANES)], wg.at[j], sem_b.at[0]))
            cps.append(pltpu.make_async_copy(wu_hbm.at[:, pl.ds(j * LANES, LANES)], wu.at[j], sem_b.at[1]))
        for j in range(KT):
            cps.append(pltpu.make_async_copy(wd_hbm.at[:, pl.ds(j * LANES, LANES)], wd.at[j], sem_b.at[2]))
        return cps

    def start_pair(g, slot):
        for c in range(3):
            raw_copy(g, slot, c).start()
        x1_copy(g).start()

    for i in range(n_x0):
        x0_copy(i).start()
    start_pair(0, 0)

    wo32, wg32, wu32, wd32 = (r.bitcast(U32) for r in (wo, wg, wu, wd))
    w_r = wr_ref[...].astype(F32)
    lane8 = lax.broadcasted_iota(jnp.int32, (M, LANES), 1)

    def router(racc, xn_rows, grp):
        r = _rnd(jnp.sum(xn_rows * w_r, axis=-1, keepdims=True))
        return tuple(jnp.where(lane8 + LANES * i == grp, r, a) for i, a in enumerate(racc))

    def w_pair(g):
        return jnp.concatenate([_b16(wqkv[g, j]) for j in range(6)], axis=1)

    def head_and_pos(i):
        head = jnp.where(i < 2 * seg, i // seg, (i - 2 * seg) // M)
        j = i % seg
        pos = jnp.where(i < 2 * seg, jnp.where(j < M, j, j + M), i % M + M)
        return head, pos

    qh, qp = head_and_pos(lax.broadcasted_iota(jnp.int32, (R, R), 0))
    kh, kp = head_and_pos(lax.broadcasted_iota(jnp.int32, (R, R), 1))
    visible = (qp < M) | (qp >= kp)
    fill_ref[...] = jnp.where(qh == kh, jnp.where(visible, 0.0, NEG), -jnp.inf).astype(F32)

    n_r = n_seg * (seg // M) // LANES
    racc = tuple(jnp.zeros((M, LANES), F32) for _ in range(n_r))
    with jax.named_scope("ln0"):
        for i in range(n_x0):
            x0_copy(i).wait()
            if i == n_x0 - 1:
                for g in range(1, slots):
                    start_pair(g, g)
            for s in range(i * (n_seg // n_x0), (i + 1) * (n_seg // n_x0), 2):
                xs = jnp.concatenate([xraw[s, 0:M, :].astype(F32), xraw[s + 1, 0:M, :].astype(F32)], axis=0)
                y = _layernorm(xs)
                yb = y.astype(BF16)
                for k in range(KT):
                    xa[k, pl.ds(s * (M // 2), M), :] = pltpu.bitcast(yb[:, k * LANES:(k + 1) * LANES], U32)
                for t in range(2):
                    xn[s + t, 0:M, :] = y[t * M:(t + 1) * M].astype(BF16)
                    base[s + t, 0:M, :] = xs[t * M:(t + 1) * M] + y[t * M:(t + 1) * M]
                    racc = router(racc, y[t * M:(t + 1) * M], (s + t) * (seg // M))

    def phase_a(g, racc):
        slot = g % slots
        for c in range(3):
            raw_copy(g, slot, c).wait()
        x1_copy(g).wait()

        for t in range(segs_per):
            s = g * segs_per + t
            xs = xraw[s, M:seg, :].astype(F32)
            y = _layernorm(xs)
            xn[s, M:seg, :] = y.astype(BF16)
            base[s, M:seg, :] = xs + y
            for u in range(1, seg // M):
                racc = router(racc, y[(u - 1) * M:u * M], s * (seg // M) + u)

        lhs = jnp.concatenate([_b16(xa[k]) for k in range(KT)], axis=1)
        for c in range(3):
            ev = raw[slot, c, pl.ds(0, D // 2, stride=2), :]
            od = raw[slot, c, pl.ds(1, D // 2, stride=2), :]
            wa = (ev & np.uint32(0xFFFF)) | (od << 16)
            wb = (ev >> 16) | (od & np.uint32(0xFFFF0000))
            wqkv[g, 2 * c] = wa
            wqkv[g, 2 * c + 1] = wb
            res = jnp.dot(lhs, jnp.concatenate([_b16(wa), _b16(wb)], axis=1), preferred_element_type=F32)
            a = res[:, :LANES].reshape(n_seg, M, LANES)
            b = res[:, LANES:].reshape(n_seg, M, LANES)
            sq[g, c] = pltpu.bitcast(jnp.concatenate([a, b], axis=1).astype(BF16), U32)

        @pl.when(g + slots < n_pair)
        def _():
            start_pair(g + slots, slot)

        @pl.when(g < KT)
        def _():
            wo_copy(g).start()

        return racc

    with jax.named_scope("phaseA"):
        racc = lax.fori_loop(0, n_pair, phase_a, racc)
    for j in range(KT):
        wo_copy(j).wait()
    for cp in b_copies():
        cp.start()

    skip = cfg.get("skip", ())

    def step(s, mem):
        xs = xn[s]
        h = jnp.concatenate([mem, xs.astype(F32)[M:]], axis=0).astype(BF16)
        qkv, probs, outs = {}, {}, {}

        def proj(g):
            res = jnp.dot(h, w_pair(g), preferred_element_type=F32)
            qkv[g] = [
                jnp.concatenate([res[:, (2 * c) * LANES:(2 * c + 1) * LANES],
                                 res[:, (2 * c + 1) * LANES:(2 * c + 2) * LANES],
                                 _b16(sq[g, c, s]).astype(F32)], axis=0).astype(BF16)
                for c in range(3)]

        def qk(g):
            q, k, v = qkv.pop(g)
            if "qk" in skip:
                probs[g] = ((q + k)[:, :R], None, v)
                return
            sc = lax.dot_general(q, k, (((1,), (1,)), ((), ())), preferred_element_type=F32) * scale
            if "sm" in skip:
                probs[g] = (sc.astype(BF16), None, v)
                return
            fill = fill_ref[...]
            sc = jnp.where(fill == 0.0, sc, fill)
            e = jnp.exp(sc - jnp.max(sc, axis=-1, keepdims=True))
            probs[g] = (e.astype(BF16), 1.0 / jnp.sum(e, axis=-1, keepdims=True), v)

        def pv(g):
            e, inv, v = probs.pop(g)
            if "pv" in skip:
                o = v.astype(F32) + jnp.sum(e.astype(F32), axis=-1, keepdims=True)
            else:
                o = jnp.dot(e, v, preferred_element_type=F32)
            if inv is not None:
                o = o * inv
            so[2 * g, s] = o[2 * seg:2 * seg + M]
            so[2 * g + 1, s] = o[2 * seg + M:]
            outs[g] = jnp.concatenate([o[:seg], o[seg:2 * seg]], axis=1)

        def oproj(g0, g1, acc):
            lhs = jnp.concatenate([outs.pop(g) for g in range(g0, g1)], axis=1).astype(BF16)
            w = jnp.concatenate([_b16(wo32[j, g0 * LANES:g1 * LANES, :]) for j in range(KT)], axis=1)
            res = jnp.dot(lhs, w, preferred_element_type=F32)
            return res if acc is None else acc + res

        acc = None
        for op in cfg["order"]:
            if op[0] == "proj":
                proj(op[1])
            elif op[0] == "qk":
                qk(op[1])
            elif op[0] == "pv":
                pv(op[1])
            else:
                acc = oproj(op[1], op[2], acc)
        base[s, M:seg, :] = base[s, M:seg, :] + acc[M:]
        return acc[:M]

    with jax.named_scope("phaseB"):
        lax.fori_loop(0, n_seg, step, mem0_ref[0].astype(F32), unroll=cfg.get("unroll", 1))

    tok = [lax.broadcasted_iota(jnp.int32, (M, LANES), 0) + M * (lane8 + LANES * i) for i in range(n_r)]
    keys = [jnp.where(a != a, -jnp.inf, a) for a in racc]
    big = np.int32(n_seg * seg)

    def pick(keys, cand):
        best = jnp.max(functools.reduce(jnp.maximum, [jnp.where(c, k, -jnp.inf) for k, c in zip(keys, cand)]))
        return jnp.min(functools.reduce(
            jnp.minimum, [jnp.where(c & (k == best), t, big) for k, t, c in zip(keys, tok, cand)]))

    i0 = pick(keys, [t >= 0 for t in tok])
    i1 = pick(keys, [t != i0 for t in tok])
    row = lax.broadcasted_iota(jnp.int32, (seg, D), 0)
    row16 = lax.broadcasted_iota(jnp.int32, (2 * M, D), 0)
    x_sel = jnp.zeros((2 * M, D), F32)
    for n, i in enumerate((i0, i1)):
        blk = xn[i // seg].astype(F32)
        x_sel = jnp.where(row16 == n, jnp.sum(jnp.where(row == i % seg, blk, 0.0), axis=0, keepdims=True), x_sel)
    gate_r = jax.nn.sigmoid(_rnd(jnp.sum(x_sel * w_r, axis=-1, keepdims=True)))
    x_sel = x_sel.astype(BF16)
    for cp in b_copies():
        cp.wait()
    gt = jnp.dot(x_sel, jnp.concatenate([_b16(wg32[j]) for j in range(FT)], axis=1), preferred_element_type=F32)
    up = jnp.dot(x_sel, jnp.concatenate([_b16(wu32[j]) for j in range(FT)], axis=1), preferred_element_type=F32)
    hid = (gt * jax.nn.sigmoid(gt) * up).astype(BF16)
    y = jnp.dot(hid, jnp.concatenate([_b16(wd32[j]) for j in range(KT)], axis=1), preferred_element_type=F32) * gate_r
    for n, i in enumerate((i0, i1)):
        base[i // seg] = base[i // seg] + jnp.where(row == i % seg, y[n:n + 1], 0.0)

    cs = cfg["c_segs"]
    n_chunk = n_seg // cs

    def out_copy(c):
        return pltpu.make_async_copy(xraw.at[pl.ds(c * cs, cs)], out_hbm.at[pl.ds(c * cs, cs)], sem_out.at[c])

    def phase_c(c, carry):
        s0 = c * cs
        lhs = jnp.concatenate(
            [so[hd, pl.ds(s0, cs)].reshape(cs * M, LANES) for hd in range(2 * n_pair)], axis=1).astype(BF16)
        w = jnp.concatenate([_b16(wo32[j]) for j in range(KT)], axis=1)
        res = jnp.dot(lhs, w, preferred_element_type=F32).reshape(cs, M, D)
        b = base[pl.ds(s0, cs)]
        xraw[pl.ds(s0, cs)] = jnp.concatenate([b[:, :M] + res, b[:, M:]], axis=1).astype(BF16)
        out_copy(c).start()
        return carry

    with jax.named_scope("phaseC"):
        lax.fori_loop(0, n_chunk, phase_c, 0)
    for c in range(n_chunk):
        out_copy(c).wait()


def _order(n_pair=16, lag_qk=1, lag_pv=2, cuts=(8, 14, 16)):
    ops = []
    tail = [("oproj", a, b) for a, b in zip((0,) + tuple(cuts[:-1]), cuts)]
    for t in range(n_pair + lag_pv):
        if t < n_pair:
            ops.append(("proj", t))
        elif tail:
            ops.append(tail.pop(0))
        if 0 <= t - lag_pv < n_pair:
            ops.append(("pv", t - lag_pv))
        if 0 <= t - lag_qk < n_pair:
            ops.append(("qk", t - lag_qk))
    return tuple(ops + tail)


DEFAULT_CFG = dict(order=None, c_segs=16, slots=3, n_x0=4)


def make(cfg=None):
    cfg = dict(DEFAULT_CFG, **(cfg or {}))
    cfg['order'] = cfg['order'] or sched('p0-4 q0-3 p5-8 v0-3 q4-7 p9 o0-3 p10-12 v4-7 q8-11 p13-15 o4-5 v8-11 q12-15 o6-9 v12-15 o10-11 o12-15')

    @functools.partial(jax.jit, static_argnames=["A_seg_len"])
    def fn(A_x, A_mem0, A_Wq, A_Wk, A_Wv, A_Wo, A_seg_len, B_x, B_w_r, B_w_gate, B_w_up, B_w_down):
        del B_x
        B, S, D = A_x.shape
        _, H, E = A_Wq.shape
        M = A_mem0.shape[1]
        F = B_w_gate.shape[1]
        seg = A_seg_len
        n_seg = S // seg
        n_pair = H // 2
        KT, FT = D // LANES, F // LANES
        R = 2 * (seg + M)
        hbm = pl.BlockSpec(memory_space=pl.ANY)
        vmem = pl.BlockSpec(memory_space=pltpu.VMEM)
        out = pl.pallas_call(
            functools.partial(_kernel, cfg=cfg),
            out_shape=jax.ShapeDtypeStruct((n_seg, seg, D), BF16),
            in_specs=[hbm, vmem, hbm, hbm, hbm, hbm, vmem, hbm, hbm, hbm],
            out_specs=hbm,
            scratch_shapes=[
                pltpu.VMEM((n_seg, seg, D), BF16),
                pltpu.VMEM((n_seg, seg, D), BF16),
                pltpu.VMEM((KT, n_seg * M // 2, LANES), U32),
                pltpu.VMEM((n_seg, seg, D), F32),
                pltpu.VMEM((cfg["slots"], 3, D, LANES), U32),
                pltpu.VMEM((n_pair, 6, D // 2, LANES), U32),
                pltpu.VMEM((KT, H * E, LANES), BF16),
                pltpu.VMEM((n_pair, 3, n_seg, M, LANES), U32),
                pltpu.VMEM((H, n_seg, M, LANES), F32),
                pltpu.VMEM((FT, D, LANES), BF16),
                pltpu.VMEM((FT, D, LANES), BF16),
                pltpu.VMEM((KT, F, LANES), BF16),
                pltpu.VMEM((R, R), F32),
                pltpu.SemaphoreType.DMA((cfg["n_x0"],)),
                pltpu.SemaphoreType.DMA((n_pair,)),
                pltpu.SemaphoreType.DMA((cfg["slots"], 3)),
                pltpu.SemaphoreType.DMA((1,)),
                pltpu.SemaphoreType.DMA((3,)),
                pltpu.SemaphoreType.DMA((n_seg // cfg["c_segs"],)),
            ],
            compiler_params=pltpu.CompilerParams(
                vmem_limit_bytes=120 * 1024 * 1024, flags=cfg.get("flags")),
        )(A_x.reshape(n_seg, seg, D), A_mem0, A_Wq, A_Wk, A_Wv, A_Wo.reshape(H * E, D),
          B_w_r.reshape(1, D), B_w_gate, B_w_up, B_w_down)
        return out.reshape(B, S, D)

    return fn


def _order4(gs=4, lag_qk=1, lag_pv=2, cuts=(8, 12, 16), n_pair=16, sub=1):
    ng = n_pair // gs
    ops = []
    tail = [("oproj", a, b) for a, b in zip((0,) + tuple(cuts[:-1]), cuts)]
    for t in range(ng + lag_pv):
        if t < ng:
            ops += [("proj", t * gs + i) for i in range(gs)]
        elif tail:
            ops.append(tail.pop(0))
        if 0 <= t - lag_pv < ng:
            ops += [("pv", (t - lag_pv) * gs + i) for i in range(gs)]
        if 0 <= t - lag_qk < ng:
            ops += [("qk", (t - lag_qk) * gs + i) for i in range(gs)]
    return tuple(ops + tail)


def sched(text):
    ops = []
    for tok in text.split():
        kind = {"p": "proj", "q": "qk", "v": "pv", "o": "oproj"}[tok[0]]
        a, b = (tok[1:].split("-") * 2)[:2]
        if kind == "oproj":
            ops.append((kind, int(a), int(b) + 1))
        else:
            ops += [(kind, i) for i in range(int(a), int(b) + 1)]
    return tuple(ops)


pallas_parallel_sum__memory_aug_recurrent_mem_tr__moe_arch_mod__prompt_kernel = make()
```

```python
import functools

import jax
import jax.numpy as jnp
import numpy as np
from jax import lax
import jax.experimental.pallas as pl
import jax.experimental.pallas.tpu as pltpu

F32 = jnp.float32
BF16 = jnp.bfloat16
U32 = jnp.uint32
LANES = 128
NEG = -1000000000.0


def _rnd(v):
    return v.astype(BF16).astype(F32)


def _b16(u):
    return pltpu.bitcast(u, BF16)


def _layernorm(x):
    mean = jnp.mean(x, axis=-1, keepdims=True)
    xc = x - mean
    var = jnp.mean(xc * xc, axis=-1, keepdims=True)
    sd = _rnd(jnp.sqrt(_rnd(_rnd(var) + np.float32(np.asarray(1e-5, BF16)))))
    return _rnd(_rnd(x - _rnd(mean)) / sd)


def _kernel(x_hbm, mem0_hbm, wq_hbm, wk_hbm, wv_hbm, wo_hbm, wr_hbm, wg_hbm, wu_hbm, wd_hbm,
            out_hbm,
            xraw, xn, xa, base, raw, wqkv, wo, sq, so, wg, wu, wd, fill_ref, mem0_ref, wr_ref,
            sem_small, sem_x0, sem_x1, sem_raw, sem_wo, sem_b, sem_out, *, cfg):
    n_seg, seg, D = xraw.shape
    M = mem0_ref.shape[1]
    n_pair = wqkv.shape[0]
    slots = raw.shape[0]
    KT = D // LANES
    FT = wg.shape[0]
    R = 2 * (seg + M)
    scale = float(LANES) ** -0.5
    n_x0 = sem_x0.shape[0]

    w_u32 = [w.bitcast(U32) for w in (wq_hbm, wk_hbm, wv_hbm)]

    def raw_copy(g, slot, c):
        return pltpu.make_async_copy(w_u32[c].at[:, g, :], raw.at[slot, c], sem_raw.at[slot, c])

    def x0_copy(i):
        ss = pl.ds(i * (n_seg // n_x0), n_seg // n_x0)
        return pltpu.make_async_copy(x_hbm.at[ss, pl.ds(0, M), :], xraw.at[ss, pl.ds(0, M), :], sem_x0.at[i])

    def x1_copy(i):
        ss = pl.ds(0, 1) if i == 0 else pl.ds(1, n_seg - 1)
        return pltpu.make_async_copy(
            x_hbm.at[ss, pl.ds(M, seg - M), :], xraw.at[ss, pl.ds(M, seg - M), :], sem_x1.at[i])

    def wo_copy(j):
        return pltpu.make_async_copy(
            wo_hbm.at[:, pl.ds(pl.multiple_of(j * LANES, LANES), LANES)], wo.at[j], sem_wo.at[0])

    def b_copies():
        cps = []
        for j in range(FT):
            cps.append(pltpu.make_async_copy(wg_hbm.at[:, pl.ds(j * LANES, LANES)], wg.at[j], sem_b.at[0]))
            cps.append(pltpu.make_async_copy(wu_hbm.at[:, pl.ds(j * LANES, LANES)], wu.at[j], sem_b.at[1]))
        for j in range(KT):
            cps.append(pltpu.make_async_copy(wd_hbm.at[:, pl.ds(j * LANES, LANES)], wd.at[j], sem_b.at[2]))
        return cps

    def start_pair(g, slot):
        for c in range(3):
            raw_copy(g, slot, c).start()

    wr_copy = pltpu.make_async_copy(wr_hbm, wr_ref, sem_small.at[0])
    mem0_copy = pltpu.make_async_copy(mem0_hbm, mem0_ref, sem_small.at[1])
    for i in range(n_x0):
        x0_copy(i).start()
    raw_copy(0, 0, 0).start()

    wo32, wg32, wu32, wd32 = (r.bitcast(U32) for r in (wo, wg, wu, wd))
    lane8 = lax.broadcasted_iota(jnp.int32, (M, LANES), 1)

    def router(racc, xn_rows, grp):
        r = _rnd(jnp.sum(xn_rows * w_r, axis=-1, keepdims=True))
        return tuple(jnp.where(lane8 + LANES * i == grp, r, a) for i, a in enumerate(racc))

    def w_pair(g):
        return jnp.concatenate([_b16(wqkv[g, j]) for j in range(6)], axis=1)

    def head_and_pos(i):
        head = jnp.where(i < 2 * seg, i // seg, (i - 2 * seg) // M)
        j = i % seg
        pos = jnp.where(i < 2 * seg, jnp.where(j < M, j, j + M), i % M + M)
        return head, pos

    qh, qp = head_and_pos(lax.broadcasted_iota(jnp.int32, (R, R), 0))
    kh, kp = head_and_pos(lax.broadcasted_iota(jnp.int32, (R, R), 1))
    visible = (qp < M) | (qp >= kp)
    fill_ref[...] = jnp.where(qh == kh, jnp.where(visible, 0.0, NEG), -jnp.inf).astype(F32)

    with jax.named_scope("ln0"):
        for i in range(n_x0):
            x0_copy(i).wait()
            if i == cfg.get("kv_at", n_x0 - 1):
                raw_copy(0, 0, 1).start()
                raw_copy(0, 0, 2).start()
            for s in range(i * (n_seg // n_x0), (i + 1) * (n_seg // n_x0), 2):
                xs = jnp.concatenate([xraw[s, 0:M, :].astype(F32), xraw[s + 1, 0:M, :].astype(F32)], axis=0)
                yb = _layernorm(xs).astype(BF16)
                for k in range(KT):
                    xa[k, pl.ds(s * (M // 2), M), :] = pltpu.bitcast(yb[:, k * LANES:(k + 1) * LANES], U32)

    def project(g, slot, cs):
        lhs = jnp.concatenate([_b16(xa[k]) for k in range(KT)], axis=1)
        for c in cs:
            ev = raw[slot, c, pl.ds(0, D // 2, stride=2), :]
            od = raw[slot, c, pl.ds(1, D // 2, stride=2), :]
            wa = (ev & np.uint32(0xFFFF)) | (od << 16)
            wb = (ev >> 16) | (od & np.uint32(0xFFFF0000))
            wqkv[g, 2 * c] = wa
            wqkv[g, 2 * c + 1] = wb
            res = jnp.dot(lhs, jnp.concatenate([_b16(wa), _b16(wb)], axis=1), preferred_element_type=F32)
            a = res[:, :LANES].reshape(n_seg, M, LANES)
            b = res[:, LANES:].reshape(n_seg, M, LANES)
            sq[g, c] = pltpu.bitcast(jnp.concatenate([a, b], axis=1).astype(BF16), U32)

    with jax.named_scope("phaseA"):
        raw_copy(0, 0, 0).wait()
        start_pair(1, 1)
        project(0, 0, (0,))
        raw_copy(0, 0, 1).wait()
        raw_copy(0, 0, 2).wait()
        for g in range(2, slots):
            start_pair(g, g)
        wr_copy.start()
        mem0_copy.start()
        x1_copy(0).start()
        project(0, 0, (1, 2))
        start_pair(slots, 0)

        def phase_a(g, carry):
            slot = g % slots
            for c in range(3):
                raw_copy(g, slot, c).wait()
            project(g, slot, (0, 1, 2))

            @pl.when(g + slots < n_pair)
            def _():
                start_pair(g + slots, slot)

            @pl.when(g <= KT)
            def _():
                wo_copy(g - 1).start()

            @pl.when(g == KT + 1)
            def _():
                x1_copy(1).start()

            return carry

        lax.fori_loop(1, n_pair, phase_a, 0)
    for j in range(KT):
        wo_copy(j).wait()
    for cp in (x1_copy(0), x1_copy(1), wr_copy, mem0_copy):
        cp.wait()
    for cp in b_copies():
        cp.start()

    w_r = wr_ref[...].astype(F32).reshape(1, D)
    n_r = n_seg * (seg // M) // LANES

    def normalize(src, dst, racc):
        y = _layernorm(xraw[src].astype(F32))
        xn[dst] = y.astype(BF16)
        for u in range(seg // M):
            racc = router(racc, y[u * M:(u + 1) * M], dst * (seg // M) + u)
        return racc

    racc = normalize(0, 0, tuple(jnp.zeros((M, LANES), F32) for _ in range(n_r)))

    skip = cfg.get("skip", ())

    def step(s, carry):
        mem, racc = carry

        def rows():
            return jnp.concatenate([mem, xn[s].astype(F32)[M:]], axis=0).astype(BF16)

        h = [rows()]
        qkv, probs, outs = {}, {}, {}

        def proj(g):
            res = jnp.dot(h[0], w_pair(g), preferred_element_type=F32)
            qkv[g] = [
                jnp.concatenate([res[:, (2 * c) * LANES:(2 * c + 1) * LANES],
                                 res[:, (2 * c + 1) * LANES:(2 * c + 2) * LANES],
                                 _b16(sq[g, c, s]).astype(F32)], axis=0).astype(BF16)
                for c in range(3)]

        def qk(g):
            q, k, v = qkv.pop(g)
            if "qk" in skip:
                probs[g] = ((q + k)[:, :R], None, v)
                return
            sc = lax.dot_general(q, k, (((1,), (1,)), ((), ())), preferred_element_type=F32) * scale
            if "sm" in skip:
                probs[g] = (sc.astype(BF16), None, v)
                return
            fill = fill_ref[...]
            sc = jnp.where(fill == 0.0, sc, fill)
            e = jnp.exp(sc - jnp.max(sc, axis=-1, keepdims=True))
            probs[g] = (e.astype(BF16), 1.0 / jnp.sum(e, axis=-1, keepdims=True), v)

        def pv(g):
            e, inv, v = probs.pop(g)
            if "pv" in skip:
                o = v.astype(F32) + jnp.sum(e.astype(F32), axis=-1, keepdims=True)
            else:
                o = jnp.dot(e, v, preferred_element_type=F32)
            if inv is not None:
                o = o * inv
            so[2 * g, s] = o[2 * seg:2 * seg + M]
            so[2 * g + 1, s] = o[2 * seg + M:]
            outs[g] = jnp.concatenate([o[:seg], o[seg:2 * seg]], axis=1)

        def oproj(g0, g1, acc):
            lhs = jnp.concatenate([outs.pop(g) for g in range(g0, g1)], axis=1).astype(BF16)
            w = jnp.concatenate([_b16(wo32[j, g0 * LANES:g1 * LANES, :]) for j in range(KT)], axis=1)
            res = jnp.dot(lhs, w, preferred_element_type=F32)
            return res if acc is None else acc + res

        acc = None
        for op in cfg["order"]:
            if op[0] == "proj":
                proj(op[1])
            elif op[0] == "qk":
                qk(op[1])
            elif op[0] == "pv":
                pv(op[1])
            elif op[0] == "norm":
                base[s] = xraw[s].astype(F32) + xn[s].astype(F32)
                racc = normalize(jnp.minimum(s + 1, n_seg - 1), jnp.minimum(s + 1, n_seg), racc)
                h[0] = rows()
            else:
                acc = oproj(op[1], op[2], acc)
        base[s, M:seg, :] = base[s, M:seg, :] + acc[M:]
        return acc[:M], racc

    with jax.named_scope("phaseB"):
        _, racc = lax.fori_loop(0, n_seg, step, (mem0_ref[0].astype(F32), racc), unroll=cfg.get("unroll", 1))

    for cp in b_copies():
        cp.wait()

    cs = cfg["c_segs"]
    n_chunk = n_seg // cs
    KG = cfg.get("kg", 4)

    def out_main():
        return pltpu.make_async_copy(
            xraw.at[:, pl.ds(M, seg - M), :], out_hbm.at[:, pl.ds(M, seg - M), :], sem_out.at[n_chunk])

    def out_head(c):
        ss = pl.ds(c * cs, cs)
        return pltpu.make_async_copy(xraw.at[ss, pl.ds(0, M), :], out_hbm.at[ss, pl.ds(0, M), :], sem_out.at[c])

    def ffn():
        tok = [lax.broadcasted_iota(jnp.int32, (M, LANES), 0) + M * (lane8 + LANES * i) for i in range(n_r)]
        keys = [jnp.where(a != a, -jnp.inf, a) for a in racc]
        big = np.int32(n_seg * seg)

        def pick(cand):
            best = jnp.max(functools.reduce(jnp.maximum, [jnp.where(c, k, -jnp.inf) for k, c in zip(keys, cand)]))
            return jnp.min(functools.reduce(
                jnp.minimum, [jnp.where(c & (k == best), t, big) for k, t, c in zip(keys, tok, cand)]))

        i0 = pick([t >= 0 for t in tok])
        i1 = pick([t != i0 for t in tok])
        row = lax.broadcasted_iota(jnp.int32, (seg, D), 0)
        row16 = lax.broadcasted_iota(jnp.int32, (2 * M, D), 0)
        x_sel = jnp.zeros((2 * M, D), F32)
        for n, i in enumerate((i0, i1)):
            blk = xn[i // seg].astype(F32)
            x_sel = jnp.where(row16 == n, jnp.sum(jnp.where(row == i % seg, blk, 0.0), axis=0, keepdims=True), x_sel)
        gate_r = jax.nn.sigmoid(_rnd(jnp.sum(x_sel * w_r, axis=-1, keepdims=True)))
        for _ in range(cfg.get("ffn_delay", 0)):
            yield

        def small(lhs, ref, j, n_k):
            acc = None
            for k0 in range(0, n_k, KG):
                k1 = min(k0 + KG, n_k)
                part = jnp.dot(lhs[:, k0 * LANES:k1 * LANES].astype(BF16),
                               _b16(ref[j, k0 * LANES // 2:k1 * LANES // 2, :]), preferred_element_type=F32)
                acc = part if acc is None else acc + part
                yield
            return acc

        hid = []
        for j in range(FT):
            gt = yield from small(x_sel, wg32, j, KT)
            up = yield from small(x_sel, wu32, j, KT)
            hid.append(gt * jax.nn.sigmoid(gt) * up)
        hid = jnp.concatenate(hid, axis=1)
        ys = []
        for j in range(KT):
            ys.append((yield from small(hid, wd32, j, FT)))
        y = jnp.concatenate(ys, axis=1) * gate_r
        for n, i in enumerate((i0, i1)):
            base[i // seg] = base[i // seg] + jnp.where(row == i % seg, y[n:n + 1], 0.0)

    if cfg.get("only_b"):
        xraw[0] = (base[0] + so[0, 0:4].reshape(seg, LANES)[:, 0:1] + racc[0][0:1, 0:1] + racc[1][0:1, 0:1]).astype(BF16)
        out_main().start()
        out_main().wait()
        return
    with jax.named_scope("phaseC"):
        state = dict(routed=False, early=0)

        def side_work():
            yield from ffn()
            state["routed"] = True
            for s0 in range(0, n_seg, cfg.get("cvt", 1)):
                ss = pl.ds(s0, cfg.get("cvt", 1))
                xraw[ss, M:seg, :] = base[ss, M:seg, :].astype(BF16)
                yield
            out_main().start()

        def side_work2():
            for c in range(state["early"]):
                for s0 in range(c * cs, (c + 1) * cs, 2):
                    ss = pl.ds(s0, 2)
                    xraw[ss, 0:M, :] = base[ss, 0:M, :].astype(BF16)
                    yield
                out_head(c).start()

        work = [side_work(), side_work2()]
        for c in range(n_chunk):
            ss = pl.ds(c * cs, cs)
            direct = state["routed"]
            if not direct:
                state["early"] = c + 1
            lhs = [jnp.concatenate([so[hd, ss].reshape(cs * M, LANES) for hd in range(k0, k0 + KG)],
                                   axis=1).astype(BF16) for k0 in range(0, 2 * n_pair, KG)]
            for j in range(KT):
                acc = None
                for q, k0 in enumerate(range(0, 2 * n_pair, KG)):
                    part = jnp.dot(lhs[q], _b16(wo32[j, k0 * LANES // 2:(k0 + KG) * LANES // 2, :]),
                                   preferred_element_type=F32)
                    acc = part if acc is None else acc + part
                    for _ in range(cfg.get("side2", 2) if state["routed"] else cfg.get("ffn_per", 1)):
                        if work and (len(work) > 1 or direct) and next(work[0], "done") == "done":
                            work.pop(0)
                cols = pl.ds(j * LANES, LANES)
                res = base[ss, 0:M, cols] + acc.reshape(cs, M, LANES)
                if direct:
                    xraw[ss, 0:M, cols] = res.astype(BF16)
                else:
                    base[ss, 0:M, cols] = res
            if direct:
                out_head(c).start()
        assert not work
    out_main().wait()
    for c in range(n_chunk):
        out_head(c).wait()


def _order(n_pair=16, lag_qk=1, lag_pv=2, cuts=(8, 14, 16)):
    ops = []
    tail = [("oproj", a, b) for a, b in zip((0,) + tuple(cuts[:-1]), cuts)]
    for t in range(n_pair + lag_pv):
        if t < n_pair:
            ops.append(("proj", t))
        elif tail:
            ops.append(tail.pop(0))
        if 0 <= t - lag_pv < n_pair:
            ops.append(("pv", t - lag_pv))
        if 0 <= t - lag_qk < n_pair:
            ops.append(("qk", t - lag_qk))
    return tuple(ops + tail)


DEFAULT_CFG = dict(order=None, c_segs=8, slots=3, ffn_delay=16, n_x0=4)


def make(cfg=None):
    cfg = dict(DEFAULT_CFG, **(cfg or {}))
    cfg['order'] = cfg['order'] or sched('p0-2 n p3-5 q0-3 p6-8 q4-7 p9 v0-3 o0-1 p10-12 o3 o2 q8-11 p13 v4-7 p14-15 o4-5 v8-11 q12-15 o6-10 v12-15 o11 o12-15')

    @functools.partial(jax.jit, static_argnames=["A_seg_len"])
    def fn(A_x, A_mem0, A_Wq, A_Wk, A_Wv, A_Wo, A_seg_len, B_x, B_w_r, B_w_gate, B_w_up, B_w_down):
        del B_x
        B, S, D = A_x.shape
        _, H, E = A_Wq.shape
        M = A_mem0.shape[1]
        F = B_w_gate.shape[1]
        seg = A_seg_len
        n_seg = S // seg
        n_pair = H // 2
        KT, FT = D // LANES, F // LANES
        R = 2 * (seg + M)
        hbm = pl.BlockSpec(memory_space=pl.ANY)
        vmem = pl.BlockSpec(memory_space=pltpu.VMEM)
        out = pl.pallas_call(
            functools.partial(_kernel, cfg=cfg),
            out_shape=jax.ShapeDtypeStruct((n_seg, seg, D), BF16),
            in_specs=[hbm] * 10,
            out_specs=hbm,
            scratch_shapes=[
                pltpu.VMEM((n_seg, seg, D), BF16),
                pltpu.VMEM((n_seg + 1, seg, D), BF16),
                pltpu.VMEM((KT, n_seg * M // 2, LANES), U32),
                pltpu.VMEM((n_seg, seg, D), F32),
                pltpu.VMEM((cfg["slots"], 3, D, LANES), U32),
                pltpu.VMEM((n_pair, 6, D // 2, LANES), U32),
                pltpu.VMEM((KT, H * E, LANES), BF16),
                pltpu.VMEM((n_pair, 3, n_seg, M, LANES), U32),
                pltpu.VMEM((H, n_seg, M, LANES), F32),
                pltpu.VMEM((FT, D, LANES), BF16),
                pltpu.VMEM((FT, D, LANES), BF16),
                pltpu.VMEM((KT, F, LANES), BF16),
                pltpu.VMEM((R, R), F32),
                pltpu.VMEM((B, M, D), BF16),
                pltpu.VMEM((D,), BF16),
                pltpu.SemaphoreType.DMA((2,)),
                pltpu.SemaphoreType.DMA((cfg["n_x0"],)),
                pltpu.SemaphoreType.DMA((2,)),
                pltpu.SemaphoreType.DMA((cfg["slots"], 3)),
                pltpu.SemaphoreType.DMA((1,)),
                pltpu.SemaphoreType.DMA((3,)),
                pltpu.SemaphoreType.DMA((n_seg // cfg["c_segs"] + 1,)),
            ],
            compiler_params=pltpu.CompilerParams(
                vmem_limit_bytes=120 * 1024 * 1024, flags=cfg.get("flags"),
                disable_bounds_checks=cfg.get("nobc", True)),
        )(A_x.reshape(n_seg, seg, D), A_mem0, A_Wq, A_Wk, A_Wv, A_Wo.reshape(H * E, D),
          B_w_r, B_w_gate, B_w_up, B_w_down)
        return out.reshape(B, S, D)

    return fn


def _order4(gs=4, lag_qk=1, lag_pv=2, cuts=(8, 12, 16), n_pair=16, sub=1):
    ng = n_pair // gs
    ops = []
    tail = [("oproj", a, b) for a, b in zip((0,) + tuple(cuts[:-1]), cuts)]
    for t in range(ng + lag_pv):
        if t < ng:
            ops += [("proj", t * gs + i) for i in range(gs)]
        elif tail:
            ops.append(tail.pop(0))
        if 0 <= t - lag_pv < ng:
            ops += [("pv", (t - lag_pv) * gs + i) for i in range(gs)]
        if 0 <= t - lag_qk < ng:
            ops += [("qk", (t - lag_qk) * gs + i) for i in range(gs)]
    return tuple(ops + tail)


def sched(text):
    ops = []
    for tok in text.split():
        if tok == "n":
            ops.append(("norm",))
            continue
        kind = {"p": "proj", "q": "qk", "v": "pv", "o": "oproj"}[tok[0]]
        a, b = (tok[1:].split("-") * 2)[:2]
        if kind == "oproj":
            ops.append((kind, int(a), int(b) + 1))
        else:
            ops += [(kind, i) for i in range(int(a), int(b) + 1)]
    return tuple(ops)


pallas_parallel_sum__memory_aug_recurrent_mem_tr__moe_arch_mod__prompt_kernel = make()
```

```python
import functools

import jax
import jax.numpy as jnp
import numpy as np
from jax import lax
import jax.experimental.pallas as pl
import jax.experimental.pallas.tpu as pltpu

F32 = jnp.float32
BF16 = jnp.bfloat16
U32 = jnp.uint32
LANES = 128
NEG = -1000000000.0


def _rnd(v):
    return v.astype(BF16).astype(F32)


def _b16(u):
    return pltpu.bitcast(u, BF16)


def _layernorm(x):
    mean = jnp.mean(x, axis=-1, keepdims=True)
    xc = x - mean
    var = jnp.mean(xc * xc, axis=-1, keepdims=True)
    sd = _rnd(jnp.sqrt(_rnd(_rnd(var) + np.float32(np.asarray(1e-5, BF16)))))
    return _rnd(_rnd(x - _rnd(mean)) / sd)


def _kernel(x_hbm, mem0_hbm, wq_hbm, wk_hbm, wv_hbm, wo_hbm, wr_hbm, wg_hbm, wu_hbm, wd_hbm,
            out_hbm,
            xraw, xn, xa, base, raw, wqkv, wo, sq, so, wg, wu, wd, fill_ref, mem0_ref, wr_ref,
            sem_small, sem_x0, sem_x1, sem_raw, sem_wo, sem_b, sem_out, *, cfg):
    n_seg, seg, D = xraw.shape
    M = mem0_ref.shape[1]
    n_pair = wqkv.shape[0]
    slots = raw.shape[0]
    KT = D // LANES
    FT = wg.shape[0]
    R = 2 * (seg + M)
    scale = float(LANES) ** -0.5
    n_x0 = sem_x0.shape[0]

    w_u32 = [w.bitcast(U32) for w in (wq_hbm, wk_hbm, wv_hbm)]

    def raw_copy(g, slot, c):
        return pltpu.make_async_copy(w_u32[c].at[:, g, :], raw.at[slot, c], sem_raw.at[slot, c])

    def x0_copy(i):
        ss = pl.ds(i * (n_seg // n_x0), n_seg // n_x0)
        return pltpu.make_async_copy(x_hbm.at[ss, pl.ds(0, M), :], xraw.at[ss, pl.ds(0, M), :], sem_x0.at[i])

    def x1_copy(i):
        ss = pl.ds(0, 1) if i == 0 else pl.ds(1, n_seg - 1)
        return pltpu.make_async_copy(
            x_hbm.at[ss, pl.ds(M, seg - M), :], xraw.at[ss, pl.ds(M, seg - M), :], sem_x1.at[i])

    def wo_copy(j):
        return pltpu.make_async_copy(
            wo_hbm.at[:, pl.ds(pl.multiple_of(j * LANES, LANES), LANES)], wo.at[j], sem_wo.at[0])

    def b_copies():
        cps = []
        for j in range(FT):
            cps.append(pltpu.make_async_copy(wg_hbm.at[:, pl.ds(j * LANES, LANES)], wg.at[j], sem_b.at[0]))
            cps.append(pltpu.make_async_copy(wu_hbm.at[:, pl.ds(j * LANES, LANES)], wu.at[j], sem_b.at[1]))
        for j in range(KT):
            cps.append(pltpu.make_async_copy(wd_hbm.at[:, pl.ds(j * LANES, LANES)], wd.at[j], sem_b.at[2]))
        return cps

    def start_pair(g, slot):
        for c in range(3):
            raw_copy(g, slot, c).start()

    wr_copy = pltpu.make_async_copy(wr_hbm, wr_ref, sem_small.at[0])
    mem0_copy = pltpu.make_async_copy(mem0_hbm, mem0_ref, sem_small.at[1])
    for i in range(n_x0):
        x0_copy(i).start()
    raw_copy(0, 0, 0).start()

    wo32, wg32, wu32, wd32 = (r.bitcast(U32) for r in (wo, wg, wu, wd))
    lane8 = lax.broadcasted_iota(jnp.int32, (M, LANES), 1)

    def router(racc, xn_rows, grp):
        r = _rnd(jnp.sum(xn_rows * w_r, axis=-1, keepdims=True))
        return tuple(jnp.where(lane8 + LANES * i == grp, r, a) for i, a in enumerate(racc))

    def w_pair(g):
        return jnp.concatenate([_b16(wqkv[g, j]) for j in range(6)], axis=1)

    def head_and_pos(i):
        head = jnp.where(i < 2 * seg, i // seg, (i - 2 * seg) // M)
        j = i % seg
        pos = jnp.where(i < 2 * seg, jnp.where(j < M, j, j + M), i % M + M)
        return head, pos

    qh, qp = head_and_pos(lax.broadcasted_iota(jnp.int32, (R, R), 0))
    kh, kp = head_and_pos(lax.broadcasted_iota(jnp.int32, (R, R), 1))
    visible = (qp < M) | (qp >= kp)
    fill_ref[...] = jnp.where(qh == kh, jnp.where(visible, 0.0, NEG), -jnp.inf).astype(F32)

    with jax.named_scope("ln0"):
        for i in range(n_x0):
            x0_copy(i).wait()
            if i == cfg.get("kv_at", n_x0 - 1):
                raw_copy(0, 0, 1).start()
                raw_copy(0, 0, 2).start()
            for s in range(i * (n_seg // n_x0), (i + 1) * (n_seg // n_x0), 2):
                xs = jnp.concatenate([xraw[s, 0:M, :].astype(F32), xraw[s + 1, 0:M, :].astype(F32)], axis=0)
                yb = _layernorm(xs).astype(BF16)
                for k in range(KT):
                    xa[k, pl.ds(s * (M // 2), M), :] = pltpu.bitcast(yb[:, k * LANES:(k + 1) * LANES], U32)

    def project(g, slot, cs):
        lhs = jnp.concatenate([_b16(xa[k]) for k in range(KT)], axis=1)
        for c in cs:
            ev = raw[slot, c, pl.ds(0, D // 2, stride=2), :]
            od = raw[slot, c, pl.ds(1, D // 2, stride=2), :]
            wa = (ev & np.uint32(0xFFFF)) | (od << 16)
            wb = (ev >> 16) | (od & np.uint32(0xFFFF0000))
            wqkv[g, 2 * c] = wa
            wqkv[g, 2 * c + 1] = wb
            res = jnp.dot(lhs, jnp.concatenate([_b16(wa), _b16(wb)], axis=1), preferred_element_type=F32)
            a = res[:, :LANES].reshape(n_seg, M, LANES)
            b = res[:, LANES:].reshape(n_seg, M, LANES)
            sq[g, c] = pltpu.bitcast(jnp.concatenate([a, b], axis=1).astype(BF16), U32)

    with jax.named_scope("phaseA"):
        raw_copy(0, 0, 0).wait()
        start_pair(1, 1)
        project(0, 0, (0,))
        raw_copy(0, 0, 1).wait()
        raw_copy(0, 0, 2).wait()
        for g in range(2, slots):
            start_pair(g, g)
        wr_copy.start()
        mem0_copy.start()
        x1_copy(0).start()
        project(0, 0, (1, 2))
        start_pair(slots, 0)

        def phase_a(g, carry):
            slot = g % slots
            for c in range(3):
                raw_copy(g, slot, c).wait()
            project(g, slot, (0, 1, 2))

            @pl.when(g + slots < n_pair)
            def _():
                start_pair(g + slots, slot)

            @pl.when(g <= KT)
            def _():
                wo_copy(g - 1).start()

            @pl.when(g == KT + 1)
            def _():
                x1_copy(1).start()

            return carry

        lax.fori_loop(1, n_pair, phase_a, 0)
    for j in range(KT):
        wo_copy(j).wait()
    for cp in (x1_copy(0), x1_copy(1), wr_copy, mem0_copy):
        cp.wait()
    for cp in b_copies():
        cp.start()

    w_r = wr_ref[...].astype(F32).reshape(1, D)
    n_r = n_seg * (seg // M) // LANES

    def normalize(src, dst, racc):
        y = _layernorm(xraw[src].astype(F32))
        xn[dst] = y.astype(BF16)
        for u in range(seg // M):
            racc = router(racc, y[u * M:(u + 1) * M], dst * (seg // M) + u)
        return racc

    racc = normalize(0, 0, tuple(jnp.zeros((M, LANES), F32) for _ in range(n_r)))

    skip = cfg.get("skip", ())

    def step(s, carry, u=0):
        mem, racc = carry

        def rows():
            return jnp.concatenate([mem, xn[s].astype(F32)[M:]], axis=0).astype(BF16)

        h = [rows()]
        qkv, probs, outs, done = {}, {}, {}, []

        def proj(g):
            if u > 0 and g in cfg.get("ksplit", ()):
                w = w_pair(g)
                hf = jnp.concatenate([mem, xn[s].astype(F32)[M:]], axis=0)
                nsp = cfg.get("nsp", 2)
                res = None
                for i in range(nsp):
                    cols = slice(i * D // nsp, (i + 1) * D // nsp)
                    part = jnp.dot(hf[:, cols].astype(BF16), w[cols], preferred_element_type=F32)
                    res = part if res is None else res + part
            else:
                res = jnp.dot(h[0], w_pair(g), preferred_element_type=F32)
            qkv[g] = [
                jnp.concatenate([res[:, (2 * c) * LANES:(2 * c + 1) * LANES],
                                 res[:, (2 * c + 1) * LANES:(2 * c + 2) * LANES],
                                 _b16(sq[g, c, s]).astype(F32)], axis=0).astype(BF16)
                for c in range(3)]

        def qk(g):
            q, k, v = qkv.pop(g)
            if "qk" in skip:
                probs[g] = ((q + k)[:, :R], None, v)
                return
            sc = lax.dot_general(q, k, (((1,), (1,)), ((), ())), preferred_element_type=F32) * scale
            if "sm" in skip:
                probs[g] = (sc.astype(BF16), None, v)
                return
            fill = fill_ref[...]
            sc = jnp.where(fill == 0.0, sc, fill)
            e = jnp.exp(sc - jnp.max(sc, axis=-1, keepdims=True))
            probs[g] = (e.astype(BF16), 1.0 / jnp.sum(e, axis=-1, keepdims=True), v)

        def pv(g):
            e, inv, v = probs.pop(g)
            if "pv" in skip:
                o = v.astype(F32) + jnp.sum(e.astype(F32), axis=-1, keepdims=True)
            else:
                o = jnp.dot(e, v, preferred_element_type=F32)
            if inv is not None:
                o = o * inv
            so[2 * g, s] = o[2 * seg:2 * seg + M]
            so[2 * g + 1, s] = o[2 * seg + M:]
            done.append(g)
            outs[g] = jnp.concatenate([o[:seg], o[seg:2 * seg]], axis=1)

        def oproj(g0, g1, acc):
            lhs = jnp.concatenate([outs.pop(g) for g in range(g0, g1)], axis=1).astype(BF16)
            nsp = cfg.get("osplit", 1) if not outs and len(done) == n_pair else 1
            res = jnp.concatenate([jnp.dot(
                lhs, jnp.concatenate([_b16(wo32[j, g0 * LANES:g1 * LANES, :])
                                      for j in range(i * KT // nsp, (i + 1) * KT // nsp)], axis=1),
                preferred_element_type=F32) for i in range(nsp)], axis=1)
            return res if acc is None else acc + res

        acc = None
        for op in (cfg.get("order2") if u and cfg.get("order2") else cfg["order"]):
            if op[0] == "proj":
                proj(op[1])
            elif op[0] == "qk":
                qk(op[1])
            elif op[0] == "pv":
                pv(op[1])
            elif op[0] == "norm":
                base[s] = xraw[s].astype(F32) + xn[s].astype(F32)
                racc = normalize(jnp.minimum(s + 1, n_seg - 1), jnp.minimum(s + 1, n_seg), racc)
                h[0] = rows()
            else:
                acc = oproj(op[1], op[2], acc)
        base[s, M:seg, :] = base[s, M:seg, :] + acc[M:]
        return acc[:M], racc

    with jax.named_scope("phaseB"):
        U = cfg.get("unroll", 1)

        def steps(i, carry):
            for u in range(U):
                carry = step(i * U + u, carry, u)
            return carry

        _, racc = lax.fori_loop(0, n_seg // U, steps, (mem0_ref[0].astype(F32), racc))

    for cp in b_copies():
        cp.wait()

    cs = cfg["c_segs"]
    n_chunk = n_seg // cs
    KG = cfg.get("kg", 4)

    def out_main():
        return pltpu.make_async_copy(
            xraw.at[:, pl.ds(M, seg - M), :], out_hbm.at[:, pl.ds(M, seg - M), :], sem_out.at[n_chunk])

    def out_head(c):
        ss = pl.ds(c * cs, cs)
        return pltpu.make_async_copy(xraw.at[ss, pl.ds(0, M), :], out_hbm.at[ss, pl.ds(0, M), :], sem_out.at[c])

    def ffn():
        tok = [lax.broadcasted_iota(jnp.int32, (M, LANES), 0) + M * (lane8 + LANES * i) for i in range(n_r)]
        keys = [jnp.where(a != a, -jnp.inf, a) for a in racc]
        big = np.int32(n_seg * seg)

        def pick(cand):
            best = jnp.max(functools.reduce(jnp.maximum, [jnp.where(c, k, -jnp.inf) for k, c in zip(keys, cand)]))
            return jnp.min(functools.reduce(
                jnp.minimum, [jnp.where(c & (k == best), t, big) for k, t, c in zip(keys, tok, cand)]))

        i0 = pick([t >= 0 for t in tok])
        i1 = pick([t != i0 for t in tok])
        row = lax.broadcasted_iota(jnp.int32, (seg, D), 0)
        row16 = lax.broadcasted_iota(jnp.int32, (2 * M, D), 0)
        x_sel = jnp.zeros((2 * M, D), F32)
        for n, i in enumerate((i0, i1)):
            blk = xn[i // seg].astype(F32)
            x_sel = jnp.where(row16 == n, jnp.sum(jnp.where(row == i % seg, blk, 0.0), axis=0, keepdims=True), x_sel)
        gate_r = jax.nn.sigmoid(_rnd(jnp.sum(x_sel * w_r, axis=-1, keepdims=True)))
        for _ in range(cfg.get("ffn_delay", 0)):
            yield

        def small(lhs, ref, j, n_k):
            acc = None
            for k0 in range(0, n_k, KG):
                k1 = min(k0 + KG, n_k)
                part = jnp.dot(lhs[:, k0 * LANES:k1 * LANES].astype(BF16),
                               _b16(ref[j, k0 * LANES // 2:k1 * LANES // 2, :]), preferred_element_type=F32)
                acc = part if acc is None else acc + part
                yield
            return acc

        hid = []
        for j in range(FT):
            gt = yield from small(x_sel, wg32, j, KT)
            up = yield from small(x_sel, wu32, j, KT)
            hid.append(gt * jax.nn.sigmoid(gt) * up)
        hid = jnp.concatenate(hid, axis=1)
        ys = []
        for j in range(KT):
            ys.append((yield from small(hid, wd32, j, FT)))
        y = jnp.concatenate(ys, axis=1) * gate_r
        for n, i in enumerate((i0, i1)):
            base[i // seg] = base[i // seg] + jnp.where(row == i % seg, y[n:n + 1], 0.0)

    if cfg.get("only_b"):
        xraw[0] = (base[0] + so[0, 0:4].reshape(seg, LANES)[:, 0:1] + racc[0][0:1, 0:1] + racc[1][0:1, 0:1]).astype(BF16)
        out_main().start()
        out_main().wait()
        return
    with jax.named_scope("phaseC"):
        state = dict(routed=False, early=0)

        def side_work():
            yield from ffn()
            state["routed"] = True
            for s0 in range(0, n_seg, cfg.get("cvt", 1)):
                ss = pl.ds(s0, cfg.get("cvt", 1))
                xraw[ss, M:seg, :] = base[ss, M:seg, :].astype(BF16)
                yield
            out_main().start()

        def side_work2():
            for c in range(state["early"]):
                for s0 in range(c * cs, (c + 1) * cs, 2):
                    ss = pl.ds(s0, 2)
                    xraw[ss, 0:M, :] = base[ss, 0:M, :].astype(BF16)
                    yield
                out_head(c).start()

        work = [side_work(), side_work2()]
        for c in range(n_chunk):
            ss = pl.ds(c * cs, cs)
            direct = state["routed"]
            if not direct:
                state["early"] = c + 1
            lhs = [jnp.concatenate([so[hd, ss].reshape(cs * M, LANES) for hd in range(k0, k0 + KG)],
                                   axis=1).astype(BF16) for k0 in range(0, 2 * n_pair, KG)]
            for j in range(KT):
                acc = None
                for q, k0 in enumerate(range(0, 2 * n_pair, KG)):
                    part = jnp.dot(lhs[q], _b16(wo32[j, k0 * LANES // 2:(k0 + KG) * LANES // 2, :]),
                                   preferred_element_type=F32)
                    acc = part if acc is None else acc + part
                    for _ in range(cfg.get("side2", 2) if state["routed"] else cfg.get("ffn_per", 1)):
                        if work and (len(work) > 1 or direct) and next(work[0], "done") == "done":
                            work.pop(0)
                cols = pl.ds(j * LANES, LANES)
                res = base[ss, 0:M, cols] + acc.reshape(cs, M, LANES)
                if direct:
                    xraw[ss, 0:M, cols] = res.astype(BF16)
                else:
                    base[ss, 0:M, cols] = res
            if direct:
                out_head(c).start()
        assert not work
    out_main().wait()
    for c in range(n_chunk):
        out_head(c).wait()


def _order(n_pair=16, lag_qk=1, lag_pv=2, cuts=(8, 14, 16)):
    ops = []
    tail = [("oproj", a, b) for a, b in zip((0,) + tuple(cuts[:-1]), cuts)]
    for t in range(n_pair + lag_pv):
        if t < n_pair:
            ops.append(("proj", t))
        elif tail:
            ops.append(tail.pop(0))
        if 0 <= t - lag_pv < n_pair:
            ops.append(("pv", t - lag_pv))
        if 0 <= t - lag_qk < n_pair:
            ops.append(("qk", t - lag_qk))
    return tuple(ops + tail)


DEFAULT_CFG = dict(order=None, c_segs=8, slots=3, ffn_delay=16, unroll=2, ksplit=(0,), nsp=4, n_x0=4)


def make(cfg=None):
    cfg = dict(DEFAULT_CFG, **(cfg or {}))
    cfg['order'] = cfg['order'] or sched('p0-2 n p3-7 q0-3 p8 q4-7 p9 v0-3 o0 p10-11 o1-2 p12 q8-11 p13 v4-7 p14 o3-5 p15 v8-11 q12-15 o6-10 v12-15 o11 o12-15')

    @functools.partial(jax.jit, static_argnames=["A_seg_len"])
    def fn(A_x, A_mem0, A_Wq, A_Wk, A_Wv, A_Wo, A_seg_len, B_x, B_w_r, B_w_gate, B_w_up, B_w_down):
        del B_x
        B, S, D = A_x.shape
        _, H, E = A_Wq.shape
        M = A_mem0.shape[1]
        F = B_w_gate.shape[1]
        seg = A_seg_len
        n_seg = S // seg
        n_pair = H // 2
        KT, FT = D // LANES, F // LANES
        R = 2 * (seg + M)
        hbm = pl.BlockSpec(memory_space=pl.ANY)
        vmem = pl.BlockSpec(memory_space=pltpu.VMEM)
        out = pl.pallas_call(
            functools.partial(_kernel, cfg=cfg),
            out_shape=jax.ShapeDtypeStruct((n_seg, seg, D), BF16),
            in_specs=[hbm] * 10,
            out_specs=hbm,
            scratch_shapes=[
                pltpu.VMEM((n_seg, seg, D), BF16),
                pltpu.VMEM((n_seg + 1, seg, D), BF16),
                pltpu.VMEM((KT, n_seg * M // 2, LANES), U32),
                pltpu.VMEM((n_seg, seg, D), F32),
                pltpu.VMEM((cfg["slots"], 3, D, LANES), U32),
                pltpu.VMEM((n_pair, 6, D // 2, LANES), U32),
                pltpu.VMEM((KT, H * E, LANES), BF16),
                pltpu.VMEM((n_pair, 3, n_seg, M, LANES), U32),
                pltpu.VMEM((H, n_seg, M, LANES), F32),
                pltpu.VMEM((FT, D, LANES), BF16),
                pltpu.VMEM((FT, D, LANES), BF16),
                pltpu.VMEM((KT, F, LANES), BF16),
                pltpu.VMEM((R, R), F32),
                pltpu.VMEM((B, M, D), BF16),
                pltpu.VMEM((D,), BF16),
                pltpu.SemaphoreType.DMA((2,)),
                pltpu.SemaphoreType.DMA((cfg["n_x0"],)),
                pltpu.SemaphoreType.DMA((2,)),
                pltpu.SemaphoreType.DMA((cfg["slots"], 3)),
                pltpu.SemaphoreType.DMA((1,)),
                pltpu.SemaphoreType.DMA((3,)),
                pltpu.SemaphoreType.DMA((n_seg // cfg["c_segs"] + 1,)),
            ],
            compiler_params=pltpu.CompilerParams(
                vmem_limit_bytes=120 * 1024 * 1024, flags=cfg.get("flags"),
                disable_bounds_checks=cfg.get("nobc", True)),
        )(A_x.reshape(n_seg, seg, D), A_mem0, A_Wq, A_Wk, A_Wv, A_Wo.reshape(H * E, D),
          B_w_r, B_w_gate, B_w_up, B_w_down)
        return out.reshape(B, S, D)

    return fn


def _order4(gs=4, lag_qk=1, lag_pv=2, cuts=(8, 12, 16), n_pair=16, sub=1):
    ng = n_pair // gs
    ops = []
    tail = [("oproj", a, b) for a, b in zip((0,) + tuple(cuts[:-1]), cuts)]
    for t in range(ng + lag_pv):
        if t < ng:
            ops += [("proj", t * gs + i) for i in range(gs)]
        elif tail:
            ops.append(tail.pop(0))
        if 0 <= t - lag_pv < ng:
            ops += [("pv", (t - lag_pv) * gs + i) for i in range(gs)]
        if 0 <= t - lag_qk < ng:
            ops += [("qk", (t - lag_qk) * gs + i) for i in range(gs)]
    return tuple(ops + tail)


def sched(text):
    ops = []
    for tok in text.split():
        if tok == "n":
            ops.append(("norm",))
            continue
        kind = {"p": "proj", "q": "qk", "v": "pv", "o": "oproj"}[tok[0]]
        a, b = (tok[1:].split("-") * 2)[:2]
        if kind == "oproj":
            ops.append((kind, int(a), int(b) + 1))
        else:
            ops += [(kind, i) for i in range(int(a), int(b) + 1)]
    return tuple(ops)


pallas_parallel_sum__memory_aug_recurrent_mem_tr__moe_arch_mod__prompt_kernel = make()
```

```python
import functools

import jax
import jax.numpy as jnp
import numpy as np
from jax import lax
import jax.experimental.pallas as pl
import jax.experimental.pallas.tpu as pltpu

F32 = jnp.float32
BF16 = jnp.bfloat16
U32 = jnp.uint32
LANES = 128
MASKED = -1000000000.0

X_CHUNKS = 4
PAIRS_PER_ITER = 2
RAW_SLOTS = 2 * PAIRS_PER_ITER
TAIL_SEGS = 8
K_GROUP = 4

STEP_ORDER = ("p0-2 n p3-7 q0-3 p8 q4-7 p9 v0-3 o0 p10-11 o1-2 p12 q8-11 p13 v4-7 p14 o3-5 p15 "
              "v8-11 q12-15 o6-10 v12-15 o11 o12-15")


def _rnd(v):
    return v.astype(BF16).astype(F32)


def _b16(u):
    return pltpu.bitcast(u, BF16)


def _dot(a, b):
    return lax.dot_general(a, b, (((1,), (0,)), ((), ())), preferred_element_type=F32)


def _layernorm(x):
    mean = jnp.mean(x, axis=-1, keepdims=True)
    xc = x - mean
    var = jnp.mean(xc * xc, axis=-1, keepdims=True)
    sd = _rnd(jnp.sqrt(_rnd(_rnd(var) + np.float32(np.asarray(1e-5, BF16)))))
    return _rnd(_rnd(x - _rnd(mean)) / sd)


def _kernel(x_hbm, mem0_hbm, wq_hbm, wk_hbm, wv_hbm, wo_hbm, wr_hbm, wg_hbm, wu_hbm, wd_hbm,
            out_hbm,
            xraw, xn, xa, base, raw, wqkv, wo, sq, so, wg, wu, wd, fill_ref, mem0_ref, wr_ref,
            sem_small, sem_x0, sem_x1, sem_raw, sem_wo, sem_ffn, sem_out):
    n_seg, seg, D = xraw.shape
    M = mem0_ref.shape[1]
    n_pair = wqkv.shape[0]
    KT = D // LANES
    FT = wg.shape[0]
    HALF = LANES // 2
    R = 2 * (seg + M)
    n_r = n_seg * (seg // M) // LANES
    n_chunk = n_seg // TAIL_SEGS
    scale = float(LANES) ** -0.5

    qkv32 = [w.bitcast(U32) for w in (wq_hbm, wk_hbm, wv_hbm)]
    wo32, wg32, wu32, wd32 = (w.bitcast(U32) for w in (wo_hbm, wg_hbm, wu_hbm, wd_hbm))

    def raw_copy(g, slot, c):
        return pltpu.make_async_copy(qkv32[c].at[:, g, :], raw.at[slot, c], sem_raw.at[slot, c])

    def start_pair(g, slot):
        for c in range(3):
            raw_copy(g, slot, c).start()

    def wait_pair(g, slot):
        for c in range(3):
            raw_copy(g, slot, c).wait()

    def x0_copy(i):
        ss = pl.ds(i * (n_seg // X_CHUNKS), n_seg // X_CHUNKS)
        return pltpu.make_async_copy(x_hbm.at[ss, pl.ds(0, M), :], xraw.at[ss, pl.ds(0, M), :], sem_x0.at[i])

    def x1_copy():
        return pltpu.make_async_copy(
            x_hbm.at[:, pl.ds(M, seg - M), :], xraw.at[:, pl.ds(M, seg - M), :], sem_x1.at[0])

    def wo_copy(j):
        return pltpu.make_async_copy(
            wo32.at[:, pl.ds(pl.multiple_of(j * LANES, LANES), LANES)], wo.at[j], sem_wo.at[0])

    def ffn_copies():
        cps = []
        for i, (src, dst) in enumerate(((wg32, wg), (wu32, wu), (wd32, wd))):
            for j in range(dst.shape[0]):
                cps.append(pltpu.make_async_copy(src.at[:, pl.ds(j * LANES, LANES)], dst.at[j], sem_ffn.at[i]))
        return cps

    def small_copies():
        return (pltpu.make_async_copy(wr_hbm, wr_ref, sem_small.at[0]),
                pltpu.make_async_copy(mem0_hbm, mem0_ref, sem_small.at[1]))

    def out_rest():
        return pltpu.make_async_copy(
            xraw.at[:, pl.ds(M, seg - M), :], out_hbm.at[:, pl.ds(M, seg - M), :], sem_out.at[n_chunk])

    def out_head(c):
        ss = pl.ds(c * TAIL_SEGS, TAIL_SEGS)
        return pltpu.make_async_copy(xraw.at[ss, pl.ds(0, M), :], out_hbm.at[ss, pl.ds(0, M), :], sem_out.at[c])

    for i in range(X_CHUNKS):
        x0_copy(i).start()
    raw_copy(0, 0, 0).start()

    def head_and_pos(i):
        head = jnp.where(i < 2 * seg, i // seg, (i - 2 * seg) // M)
        j = i % seg
        pos = jnp.where(i < 2 * seg, jnp.where(j < M, j, j + M), i % M + M)
        return head, pos

    qh, qp = head_and_pos(lax.broadcasted_iota(jnp.int32, (R, R), 0))
    kh, kp = head_and_pos(lax.broadcasted_iota(jnp.int32, (R, R), 1))
    visible = (qp < M) | (qp >= kp)
    fill_ref[...] = jnp.where(qh == kh, jnp.where(visible, 0.0, MASKED), -jnp.inf).astype(F32)

    for i in range(X_CHUNKS):
        x0_copy(i).wait()
        if i == X_CHUNKS - 1:
            raw_copy(0, 0, 1).start()
            raw_copy(0, 0, 2).start()
        for s in range(i * (n_seg // X_CHUNKS), (i + 1) * (n_seg // X_CHUNKS), 2):
            xs = jnp.concatenate([xraw[s, 0:M, :].astype(F32), xraw[s + 1, 0:M, :].astype(F32)], axis=0)
            y = _layernorm(xs).astype(BF16)
            for k in range(KT):
                xa[k, pl.ds(s * (M // 2), M), :] = pltpu.bitcast(y[:, k * LANES:(k + 1) * LANES], U32)

    def project(g, slot, which):
        lhs = jnp.concatenate([_b16(xa[k]) for k in range(KT)], axis=1)
        for c in which:
            even = raw[slot, c, pl.ds(0, D // 2, stride=2), :]
            odd = raw[slot, c, pl.ds(1, D // 2, stride=2), :]
            wa = (even & np.uint32(0xFFFF)) | (odd << 16)
            wb = (even >> 16) | (odd & np.uint32(0xFFFF0000))
            wqkv[g, 2 * c] = wa
            wqkv[g, 2 * c + 1] = wb
            res = _dot(lhs, jnp.concatenate([_b16(wa), _b16(wb)], axis=1))
            a = res[:, :LANES].reshape(n_seg, M, LANES)
            b = res[:, LANES:].reshape(n_seg, M, LANES)
            sq[g, c] = pltpu.bitcast(jnp.concatenate([a, b], axis=1).astype(BF16), U32)

    raw_copy(0, 0, 0).wait()
    start_pair(1, 1)
    project(0, 0, (0,))
    raw_copy(0, 0, 1).wait()
    raw_copy(0, 0, 2).wait()
    start_pair(2, 2)
    for cp in small_copies():
        cp.start()
    project(0, 0, (1, 2))
    wait_pair(1, 1)
    start_pair(3, 3)
    project(1, 1, (0, 1, 2))
    start_pair(RAW_SLOTS, 0)
    start_pair(RAW_SLOTS + 1, 1)

    def phase_a(i, carry):
        g0 = i * PAIRS_PER_ITER
        slot0 = (i % 2) * PAIRS_PER_ITER
        for u in range(PAIRS_PER_ITER):
            wait_pair(g0 + u, slot0 + u)
        for u in range(PAIRS_PER_ITER):
            project(g0 + u, slot0 + u, (0, 1, 2))

        @pl.when(i + 2 < n_pair // PAIRS_PER_ITER)
        def _():
            for u in range(PAIRS_PER_ITER):
                start_pair(g0 + RAW_SLOTS + u, slot0 + u)

        @pl.when(i <= KT // PAIRS_PER_ITER)
        def _():
            for u in range(PAIRS_PER_ITER):
                wo_copy((i - 1) * PAIRS_PER_ITER + u).start()

        @pl.when(i == KT // PAIRS_PER_ITER + 1)
        def _():
            x1_copy().start()

        return carry

    lax.fori_loop(1, n_pair // PAIRS_PER_ITER, phase_a, 0)
    for j in range(KT):
        wo_copy(j).wait()
    x1_copy().wait()
    for cp in small_copies():
        cp.wait()
    for cp in ffn_copies():
        cp.start()

    w_r = wr_ref[...].astype(F32).reshape(1, D)
    lane = lax.broadcasted_iota(jnp.int32, (M, LANES), 1)

    def normalize(src, dst, scores):
        y = _layernorm(xraw[src].astype(F32))
        xn[dst] = y.astype(BF16)
        for u in range(seg // M):
            r = _rnd(jnp.sum(y[u * M:(u + 1) * M] * w_r, axis=-1, keepdims=True))
            grp = dst * (seg // M) + u
            scores = tuple(jnp.where(lane + LANES * i == grp, r, a) for i, a in enumerate(scores))
        return scores

    def step(s, carry, split_first):
        mem, scores = carry

        def rows():
            return jnp.concatenate([mem, xn[s].astype(F32)[M:]], axis=0)

        h = rows().astype(BF16)
        qkv, probs, outs = {}, {}, {}
        acc = None
        for op in STEP_ORDER.split():
            if op == "n":
                base[s] = xraw[s].astype(F32) + xn[s].astype(F32)
                scores = normalize(jnp.minimum(s + 1, n_seg - 1), jnp.minimum(s + 1, n_seg), scores)
                h = rows().astype(BF16)
                continue
            g0, g1 = (int(t) for t in (op[1:].split("-") * 2)[:2])
            if op[0] == "o":
                lhs = jnp.concatenate([outs.pop(g) for g in range(g0, g1 + 1)], axis=1).astype(BF16)
                res = _dot(lhs, jnp.concatenate(
                    [_b16(wo[j, g0 * LANES:(g1 + 1) * LANES, :]) for j in range(KT)], axis=1))
                acc = res if acc is None else acc + res
                continue
            for g in range(g0, g1 + 1):
                if op[0] == "p":
                    w = jnp.concatenate([_b16(wqkv[g, j]) for j in range(6)], axis=1)
                    if g == 0 and split_first:
                        hf = rows()
                        res = None
                        for i in range(4):
                            cols = slice(i * D // 4, (i + 1) * D // 4)
                            part = _dot(hf[:, cols].astype(BF16), w[cols])
                            res = part if res is None else res + part
                    else:
                        res = _dot(h, w)
                    qkv[g] = [
                        jnp.concatenate([res[:, (2 * c) * LANES:(2 * c + 1) * LANES],
                                         res[:, (2 * c + 1) * LANES:(2 * c + 2) * LANES],
                                         _b16(sq[g, c, s]).astype(F32)], axis=0).astype(BF16)
                        for c in range(3)]
                elif op[0] == "q":
                    q, k, v = qkv.pop(g)
                    sc = lax.dot_general(q, k, (((1,), (1,)), ((), ())), preferred_element_type=F32) * scale
                    fill = fill_ref[...]
                    sc = jnp.where(fill == 0.0, sc, fill)
                    e = jnp.exp(sc - jnp.max(sc, axis=-1, keepdims=True))
                    probs[g] = (e.astype(BF16), 1.0 / jnp.sum(e, axis=-1, keepdims=True), v)
                else:
                    e, inv, v = probs.pop(g)
                    o = _dot(e, v) * inv
                    so[2 * g, s] = o[2 * seg:2 * seg + M]
                    so[2 * g + 1, s] = o[2 * seg + M:]
                    outs[g] = jnp.concatenate([o[:seg], o[seg:2 * seg]], axis=1)
        base[s, M:seg, :] = base[s, M:seg, :] + acc[M:]
        return acc[:M], scores

    def two_steps(i, carry):
        return step(2 * i + 1, step(2 * i, carry, False), True)

    scores = normalize(0, 0, tuple(jnp.zeros((M, LANES), F32) for _ in range(n_r)))
    _, scores = lax.fori_loop(0, n_seg // 2, two_steps, (mem0_ref[0].astype(F32), scores))

    for cp in ffn_copies():
        cp.wait()

    def routed_ffn():
        tok = [lax.broadcasted_iota(jnp.int32, (M, LANES), 0) + M * (lane + LANES * i) for i in range(n_r)]
        keys = [jnp.where(a != a, -jnp.inf, a) for a in scores]

        def pick(cand):
            best = jnp.max(functools.reduce(jnp.maximum, [jnp.where(c, k, -jnp.inf) for k, c in zip(keys, cand)]))
            return jnp.min(functools.reduce(jnp.minimum, [
                jnp.where(c & (k == best), t, n_seg * seg) for k, t, c in zip(keys, tok, cand)]))

        first = pick([t >= 0 for t in tok])
        second = pick([t != first for t in tok])
        row = lax.broadcasted_iota(jnp.int32, (seg, D), 0)
        slot = lax.broadcasted_iota(jnp.int32, (M, D), 0)
        x_sel = jnp.zeros((M, D), F32)
        for n, i in enumerate((first, second)):
            picked = jnp.sum(jnp.where(row == i % seg, xn[i // seg].astype(F32), 0.0), axis=0, keepdims=True)
            x_sel = jnp.where(slot == n, picked, x_sel)
        weight = jax.nn.sigmoid(_rnd(jnp.sum(x_sel * w_r, axis=-1, keepdims=True)))
        for _ in range(16):
            yield

        hidden = []
        for j in range(FT):
            gu = None
            for k in range(0, KT, 2):
                tiles = slice(k * HALF, (k + 2) * HALF)
                part = _dot(x_sel[:, k * LANES:(k + 2) * LANES],
                            jnp.concatenate([_b16(wg[j, tiles, :]), _b16(wu[j, tiles, :])], axis=1))
                gu = part if gu is None else gu + part
                yield
            gate, up = gu[:, :LANES], gu[:, LANES:]
            hidden.append(_rnd(gate * jax.nn.sigmoid(gate) * up))
        ys = []
        for j0 in range(0, KT, K_GROUP):
            acc = None
            for k in range(FT):
                part = _dot(hidden[k], jnp.concatenate(
                    [_b16(wd[j, k * HALF:(k + 1) * HALF, :]) for j in range(j0, j0 + K_GROUP)], axis=1))
                acc = part if acc is None else acc + part
                yield
            ys.append(acc)
        y = jnp.concatenate(ys, axis=1) * weight
        for n, i in enumerate((first, second)):
            base[i // seg] = base[i // seg] + jnp.where(row == i % seg, y[n:n + 1], 0.0)

    state = {"routed": False, "early": 0}

    def side_work():
        yield from routed_ffn()
        state["routed"] = True
        for s in range(n_seg):
            xraw[pl.ds(s, 1), M:seg, :] = base[pl.ds(s, 1), M:seg, :].astype(BF16)
            yield
        out_rest().start()

    def early_heads():
        for c in range(state["early"]):
            for s in range(c * TAIL_SEGS, (c + 1) * TAIL_SEGS, 2):
                xraw[pl.ds(s, 2), 0:M, :] = base[pl.ds(s, 2), 0:M, :].astype(BF16)
                yield
            out_head(c).start()

    work = [side_work(), early_heads()]
    for c in range(n_chunk):
        ss = pl.ds(c * TAIL_SEGS, TAIL_SEGS)
        direct = state["routed"]
        if not direct:
            state["early"] = c + 1
        lhs = [jnp.concatenate([so[hd, ss].reshape(TAIL_SEGS * M, LANES) for hd in range(k, k + K_GROUP)],
                               axis=1).astype(BF16) for k in range(0, 2 * n_pair, K_GROUP)]
        for j in range(KT):
            acc = None
            for i, k in enumerate(range(0, 2 * n_pair, K_GROUP)):
                part = _dot(lhs[i], _b16(wo[j, k * HALF:(k + K_GROUP) * HALF, :]))
                acc = part if acc is None else acc + part
                for _ in range(2 if state["routed"] else 1):
                    if work and (len(work) > 1 or direct) and next(work[0], "done") == "done":
                        work.pop(0)
            cols = pl.ds(j * LANES, LANES)
            res = base[ss, 0:M, cols] + acc.reshape(TAIL_SEGS, M, LANES)
            if direct:
                xraw[ss, 0:M, cols] = res.astype(BF16)
            else:
                base[ss, 0:M, cols] = res
        if direct:
            out_head(c).start()
    assert not work
    out_rest().wait()
    for c in range(n_chunk):
        out_head(c).wait()


@functools.partial(jax.jit, static_argnames=["A_seg_len"])
def pallas_parallel_sum__memory_aug_recurrent_mem_tr__moe_arch_mod__prompt_kernel(
    A_x, A_mem0, A_Wq, A_Wk, A_Wv, A_Wo, A_seg_len, B_x, B_w_r, B_w_gate, B_w_up, B_w_down,
):
    del B_x
    B, S, D = A_x.shape
    _, H, E = A_Wq.shape
    M = A_mem0.shape[1]
    F = B_w_gate.shape[1]
    seg = A_seg_len
    n_seg = S // seg
    n_pair = H // 2
    KT, FT = D // LANES, F // LANES
    R = 2 * (seg + M)
    assert (B, M, seg, H, E) == (1, 8, 32, 32, LANES) and n_seg * seg == S
    hbm = pl.BlockSpec(memory_space=pl.ANY)
    out = pl.pallas_call(
        _kernel,
        out_shape=jax.ShapeDtypeStruct((n_seg, seg, D), A_x.dtype),
        in_specs=[hbm] * 10,
        out_specs=hbm,
        scratch_shapes=[
            pltpu.VMEM((n_seg, seg, D), BF16),
            pltpu.VMEM((n_seg + 1, seg, D), BF16),
            pltpu.VMEM((KT, n_seg * M // 2, LANES), U32),
            pltpu.VMEM((n_seg, seg, D), F32),
            pltpu.VMEM((RAW_SLOTS, 3, D, LANES), U32),
            pltpu.VMEM((n_pair, 6, D // 2, LANES), U32),
            pltpu.VMEM((KT, H * E // 2, LANES), U32),
            pltpu.VMEM((n_pair, 3, n_seg, M, LANES), U32),
            pltpu.VMEM((H, n_seg, M, LANES), F32),
            pltpu.VMEM((FT, D // 2, LANES), U32),
            pltpu.VMEM((FT, D // 2, LANES), U32),
            pltpu.VMEM((KT, F // 2, LANES), U32),
            pltpu.VMEM((R, R), F32),
            pltpu.VMEM((B, M, D), BF16),
            pltpu.VMEM((D,), BF16),
            pltpu.SemaphoreType.DMA((2,)),
            pltpu.SemaphoreType.DMA((X_CHUNKS,)),
            pltpu.SemaphoreType.DMA((1,)),
            pltpu.SemaphoreType.DMA((RAW_SLOTS, 3)),
            pltpu.SemaphoreType.DMA((1,)),
            pltpu.SemaphoreType.DMA((3,)),
            pltpu.SemaphoreType.DMA((n_seg // TAIL_SEGS + 1,)),
        ],
        compiler_params=pltpu.CompilerParams(vmem_limit_bytes=120 * 1024 * 1024),
    )(A_x.reshape(n_seg, seg, D), A_mem0, A_Wq, A_Wk, A_Wv, A_Wo.reshape(H * E, D),
      B_w_r, B_w_gate, B_w_up, B_w_down)
    return out.reshape(B, S, D)
```

```python
import functools

import jax
import jax.numpy as jnp
import numpy as np
from jax import lax
import jax.experimental.pallas as pl
import jax.experimental.pallas.tpu as pltpu

F32 = jnp.float32
BF16 = jnp.bfloat16
U32 = jnp.uint32
LANES = 128
MASKED = -1000000000.0

X_CHUNKS = 4
PAIRS_PER_ITER = 2
RAW_SLOTS = 2 * PAIRS_PER_ITER
TAIL_SEGS = 8
K_GROUP = 4

STEP_ORDERS = (
    "p0-2 n p3-7 q0-3 p8 q4-7 p9 v0-3 o0 p10-11 o1 p12 o2-3 q8-11 p13 v4-7 p14-15 v8-11 o4-5 "
    "q12-15 o6-9 v12-15 o10-11 o12-15",
    "p0-2 n p3-7 q0-3 p8 q4-7 p9 v0-3 o0 p10-11 o1-2 p12 q8-11 p13 v4-7 p14 o3-5 p15 v8-11 "
    "q12-15 o6-7 o8-10 v12-15 o11 o12 o13 o14-15",
    "p0-2 n p3-5 q0-3 p6-8 q4-7 p9 v0-3 o0 p10-11 o1 p12 q8-11 p13 v4-7 p14 o2-3 p15 v8-11 o4-5 "
    "q12-15 o6-7 v12-15 o8-9 o11 o10 o12-13 o14-15",
)


def _rnd(v):
    return v.astype(BF16).astype(F32)


def _b16(u):
    return pltpu.bitcast(u, BF16)


def _dot(a, b):
    return lax.dot_general(a, b, (((1,), (0,)), ((), ())), preferred_element_type=F32)


def _layernorm(x):
    mean = jnp.mean(x, axis=-1, keepdims=True)
    xc = x - mean
    var = jnp.mean(xc * xc, axis=-1, keepdims=True)
    sd = _rnd(jnp.sqrt(_rnd(_rnd(var) + np.float32(np.asarray(1e-5, BF16)))))
    return _rnd(_rnd(x - _rnd(mean)) / sd)


def _kernel(x_hbm, mem0_hbm, wq_hbm, wk_hbm, wv_hbm, wo_hbm, wr_hbm, wg_hbm, wu_hbm, wd_hbm,
            out_hbm,
            xraw, xn, xa, base, raw, wqkv, wo, sq, so, wg, wu, wd, fill_ref, mem0_ref, wr_ref,
            sem_small, sem_x0, sem_x1, sem_raw, sem_wo, sem_ffn, sem_out):
    n_seg, seg, D = xraw.shape
    M = mem0_ref.shape[1]
    n_pair = wqkv.shape[0]
    KT = D // LANES
    FT = wg.shape[0]
    HALF = LANES // 2
    R = 2 * (seg + M)
    n_r = n_seg * (seg // M) // LANES
    n_chunk = n_seg // TAIL_SEGS
    scale = float(LANES) ** -0.5

    qkv32 = [w.bitcast(U32) for w in (wq_hbm, wk_hbm, wv_hbm)]
    wo32, wg32, wu32, wd32 = (w.bitcast(U32) for w in (wo_hbm, wg_hbm, wu_hbm, wd_hbm))

    def raw_copy(g, slot, c):
        return pltpu.make_async_copy(qkv32[c].at[:, g, :], raw.at[slot, c], sem_raw.at[slot, c])

    def start_pair(g, slot):
        for c in range(3):
            raw_copy(g, slot, c).start()

    def wait_pair(g, slot):
        for c in range(3):
            raw_copy(g, slot, c).wait()

    def x0_copy(i):
        ss = pl.ds(i * (n_seg // X_CHUNKS), n_seg // X_CHUNKS)
        return pltpu.make_async_copy(x_hbm.at[ss, pl.ds(0, M), :], xraw.at[ss, pl.ds(0, M), :], sem_x0.at[i])

    def x1_copy():
        ss = pl.ds(1, n_seg - 1)
        return pltpu.make_async_copy(
            x_hbm.at[ss, pl.ds(M, seg - M), :], xraw.at[ss, pl.ds(M, seg - M), :], sem_x1.at[0])

    def wo_copy(j):
        return pltpu.make_async_copy(
            wo32.at[:, pl.ds(pl.multiple_of(j * LANES, LANES), LANES)], wo.at[j], sem_wo.at[0])

    def ffn_copies():
        cps = []
        for i, (src, dst) in enumerate(((wg32, wg), (wu32, wu), (wd32, wd))):
            for j in range(dst.shape[0]):
                cps.append(pltpu.make_async_copy(src.at[:, pl.ds(j * LANES, LANES)], dst.at[j], sem_ffn.at[i]))
        return cps

    def small_copies():
        return (pltpu.make_async_copy(wr_hbm, wr_ref, sem_small.at[0]),
                pltpu.make_async_copy(mem0_hbm, mem0_ref, sem_small.at[1]),
                pltpu.make_async_copy(x_hbm.at[0, pl.ds(M, seg - M), :], xraw.at[0, pl.ds(M, seg - M), :],
                                      sem_small.at[2]))

    def out_rest():
        return pltpu.make_async_copy(
            xraw.at[:, pl.ds(M, seg - M), :], out_hbm.at[:, pl.ds(M, seg - M), :], sem_out.at[n_chunk])

    def out_head(c):
        ss = pl.ds(c * TAIL_SEGS, TAIL_SEGS)
        return pltpu.make_async_copy(xraw.at[ss, pl.ds(0, M), :], out_hbm.at[ss, pl.ds(0, M), :], sem_out.at[c])

    for i in range(X_CHUNKS):
        x0_copy(i).start()
    raw_copy(0, 0, 0).start()
    for cp in small_copies():
        cp.start()

    def head_and_pos(i):
        head = jnp.where(i < 2 * seg, i // seg, (i - 2 * seg) // M)
        j = i % seg
        pos = jnp.where(i < 2 * seg, jnp.where(j < M, j, j + M), i % M + M)
        return head, pos

    qh, qp = head_and_pos(lax.broadcasted_iota(jnp.int32, (R, R), 0))
    kh, kp = head_and_pos(lax.broadcasted_iota(jnp.int32, (R, R), 1))
    visible = (qp < M) | (qp >= kp)
    fill_ref[...] = jnp.where(qh == kh, jnp.where(visible, 0.0, MASKED), -jnp.inf).astype(F32)

    for i in range(X_CHUNKS):
        x0_copy(i).wait()
        if i == X_CHUNKS - 1:
            raw_copy(0, 0, 1).start()
            raw_copy(0, 0, 2).start()
        for s in range(i * (n_seg // X_CHUNKS), (i + 1) * (n_seg // X_CHUNKS), 2):
            xs = jnp.concatenate([xraw[s, 0:M, :].astype(F32), xraw[s + 1, 0:M, :].astype(F32)], axis=0)
            y = _layernorm(xs).astype(BF16)
            for k in range(KT):
                xa[k, pl.ds(s * (M // 2), M), :] = pltpu.bitcast(y[:, k * LANES:(k + 1) * LANES], U32)

    def project(g, slot, which):
        lhs = jnp.concatenate([_b16(xa[k]) for k in range(KT)], axis=1)
        for c in which:
            even = raw[slot, c, pl.ds(0, D // 2, stride=2), :]
            odd = raw[slot, c, pl.ds(1, D // 2, stride=2), :]
            wa = (even & np.uint32(0xFFFF)) | (odd << 16)
            wb = (even >> 16) | (odd & np.uint32(0xFFFF0000))
            wqkv[g, 2 * c] = wa
            wqkv[g, 2 * c + 1] = wb
            res = _dot(lhs, jnp.concatenate([_b16(wa), _b16(wb)], axis=1))
            a = res[:, :LANES].reshape(n_seg, M, LANES)
            b = res[:, LANES:].reshape(n_seg, M, LANES)
            sq[g, c] = pltpu.bitcast(jnp.concatenate([a, b], axis=1).astype(BF16), U32)

    raw_copy(0, 0, 0).wait()
    start_pair(1, 1)
    project(0, 0, (0,))
    raw_copy(0, 0, 1).wait()
    raw_copy(0, 0, 2).wait()
    start_pair(2, 2)
    project(0, 0, (1, 2))
    wait_pair(1, 1)
    for cp in small_copies():
        cp.wait()
    start_pair(3, 3)
    project(1, 1, (0, 1, 2))

    w_r = wr_ref[...].astype(F32).reshape(1, D)
    lane = lax.broadcasted_iota(jnp.int32, (M, LANES), 1)

    def normalize(s, scores):
        y = _layernorm(xraw[s].astype(F32))
        xn[s] = y.astype(BF16)
        for u in range(seg // M):
            r = _rnd(jnp.sum(y[u * M:(u + 1) * M] * w_r, axis=-1, keepdims=True))
            grp = s * (seg // M) + u
            scores = tuple(jnp.where(lane + LANES * i == grp, r, a) for i, a in enumerate(scores))
        return scores

    scores = normalize(0, tuple(jnp.zeros((M, LANES), F32) for _ in range(n_r)))
    start_pair(RAW_SLOTS, 0)
    start_pair(RAW_SLOTS + 1, 1)

    def phase_a(i, carry):
        g0 = i * PAIRS_PER_ITER
        slot0 = (i % 2) * PAIRS_PER_ITER
        for u in range(PAIRS_PER_ITER):
            wait_pair(g0 + u, slot0 + u)
        for u in range(PAIRS_PER_ITER):
            project(g0 + u, slot0 + u, (0, 1, 2))

        @pl.when(i + 2 < n_pair // PAIRS_PER_ITER)
        def _():
            for u in range(PAIRS_PER_ITER):
                start_pair(g0 + RAW_SLOTS + u, slot0 + u)

        @pl.when(i <= KT // PAIRS_PER_ITER)
        def _():
            for u in range(PAIRS_PER_ITER):
                wo_copy((i - 1) * PAIRS_PER_ITER + u).start()

        @pl.when(i == KT // PAIRS_PER_ITER + 1)
        def _():
            x1_copy().start()

        return carry

    lax.fori_loop(1, n_pair // PAIRS_PER_ITER, phase_a, 0)
    for j in range(KT):
        wo_copy(j).wait()
    x1_copy().wait()
    for cp in ffn_copies():
        cp.start()

    def step(s, carry, u):
        mem, scores = carry

        def rows():
            return jnp.concatenate([mem, xn[s].astype(F32)[M:]], axis=0)

        h = rows().astype(BF16)
        qkv, probs, outs = {}, {}, {}
        acc = None
        for op in STEP_ORDERS[u].split():
            if op == "n":
                base[s] = xraw[s].astype(F32) + xn[s].astype(F32)
                if not isinstance(s, int):
                    nxt = jnp.minimum(s + 1, n_seg - 1)
                    scores = normalize(nxt, scores)
                h = rows().astype(BF16)
                continue
            g0, g1 = (int(t) for t in (op[1:].split("-") * 2)[:2])
            if op[0] == "o":
                lhs = jnp.concatenate([outs.pop(g) for g in range(g0, g1 + 1)], axis=1).astype(BF16)
                res = _dot(lhs, jnp.concatenate(
                    [_b16(wo[j, g0 * LANES:(g1 + 1) * LANES, :]) for j in range(KT)], axis=1))
                acc = res if acc is None else acc + res
                continue
            for g in range(g0, g1 + 1):
                if op[0] == "p":
                    w = jnp.concatenate([_b16(wqkv[g, j]) for j in range(6)], axis=1)
                    if g == 0 and u > 0:
                        hf = rows()
                        res = None
                        for i in range(4):
                            cols = slice(i * D // 4, (i + 1) * D // 4)
                            part = _dot(hf[:, cols].astype(BF16), w[cols])
                            res = part if res is None else res + part
                    else:
                        res = _dot(h, w)
                    qkv[g] = [
                        jnp.concatenate([res[:, (2 * c) * LANES:(2 * c + 1) * LANES],
                                         res[:, (2 * c + 1) * LANES:(2 * c + 2) * LANES],
                                         _b16(sq[g, c, s]).astype(F32)], axis=0).astype(BF16)
                        for c in range(3)]
                elif op[0] == "q":
                    q, k, v = qkv.pop(g)
                    sc = lax.dot_general(q, k, (((1,), (1,)), ((), ())), preferred_element_type=F32) * scale
                    fill = fill_ref[...]
                    sc = jnp.where(fill == 0.0, sc, fill)
                    e = jnp.exp(sc - jnp.max(sc, axis=-1, keepdims=True))
                    total = jnp.sum(e, axis=-1, keepdims=True)
                    inv = pltpu.reciprocal(total, approx=True)
                    inv = inv * (2.0 - total * inv)
                    probs[g] = (e.astype(BF16), inv, v)
                else:
                    e, inv, v = probs.pop(g)
                    o = _dot(e, v) * inv
                    so[2 * g, s] = o[2 * seg:2 * seg + M]
                    so[2 * g + 1, s] = o[2 * seg + M:]
                    outs[g] = jnp.concatenate([o[:seg], o[seg:2 * seg]], axis=1)
        base[s, M:seg, :] = base[s, M:seg, :] + acc[M:]
        return acc[:M], scores

    unroll = len(STEP_ORDERS)

    def steps(i, carry):
        for u in range(unroll):
            carry = step(i * unroll + u, carry, u)
        return carry

    n_iter = (n_seg - 1) // unroll
    assert n_iter * unroll == n_seg - 1
    carry = lax.fori_loop(0, n_iter, steps, (mem0_ref[0].astype(F32), scores))

    for cp in ffn_copies():
        cp.wait()
    _, scores = step(n_seg - 1, carry, 0)

    def routed_ffn():
        tok = [lax.broadcasted_iota(jnp.int32, (M, LANES), 0) + M * (lane + LANES * i) for i in range(n_r)]
        keys = [jnp.where(a != a, -jnp.inf, a) for a in scores]

        def pick(cand):
            best = jnp.max(functools.reduce(jnp.maximum, [jnp.where(c, k, -jnp.inf) for k, c in zip(keys, cand)]))
            return jnp.min(functools.reduce(jnp.minimum, [
                jnp.where(c & (k == best), t, n_seg * seg) for k, t, c in zip(keys, tok, cand)]))

        first = pick([t >= 0 for t in tok])
        second = pick([t != first for t in tok])
        row = lax.broadcasted_iota(jnp.int32, (seg, D), 0)
        slot = lax.broadcasted_iota(jnp.int32, (M, D), 0)
        x_sel = jnp.zeros((M, D), F32)
        for n, i in enumerate((first, second)):
            picked = jnp.sum(jnp.where(row == i % seg, xn[i // seg].astype(F32), 0.0), axis=0, keepdims=True)
            x_sel = jnp.where(slot == n, picked, x_sel)
        weight = jax.nn.sigmoid(_rnd(jnp.sum(x_sel * w_r, axis=-1, keepdims=True)))
        for _ in range(16):
            yield

        hidden = []
        for j in range(FT):
            gu = None
            for k in range(0, KT, 2):
                tiles = slice(k * HALF, (k + 2) * HALF)
                part = _dot(x_sel[:, k * LANES:(k + 2) * LANES],
                            jnp.concatenate([_b16(wg[j, tiles, :]), _b16(wu[j, tiles, :])], axis=1))
                gu = part if gu is None else gu + part
                yield
            gate, up = gu[:, :LANES], gu[:, LANES:]
            hidden.append(_rnd(gate * jax.nn.sigmoid(gate) * up))
        ys = []
        for j0 in range(0, KT, K_GROUP):
            acc = None
            for k in range(FT):
                part = _dot(hidden[k], jnp.concatenate(
                    [_b16(wd[j, k * HALF:(k + 1) * HALF, :]) for j in range(j0, j0 + K_GROUP)], axis=1))
                acc = part if acc is None else acc + part
                yield
            ys.append(acc)
        y = jnp.concatenate(ys, axis=1) * weight
        for n, i in enumerate((first, second)):
            base[i // seg] = base[i // seg] + jnp.where(row == i % seg, y[n:n + 1], 0.0)

    state = {"routed": False, "early": 0}

    def side_work():
        yield from routed_ffn()
        state["routed"] = True
        for s in range(n_seg):
            xraw[pl.ds(s, 1), M:seg, :] = base[pl.ds(s, 1), M:seg, :].astype(BF16)
            yield
        out_rest().start()

    def early_heads():
        for c in range(state["early"]):
            for s in range(c * TAIL_SEGS, (c + 1) * TAIL_SEGS, 2):
                xraw[pl.ds(s, 2), 0:M, :] = base[pl.ds(s, 2), 0:M, :].astype(BF16)
                yield
            out_head(c).start()

    work = [side_work(), early_heads()]
    for c in range(n_chunk):
        ss = pl.ds(c * TAIL_SEGS, TAIL_SEGS)
        direct = state["routed"]
        if not direct:
            state["early"] = c + 1
        lhs = [jnp.concatenate([so[hd, ss].reshape(TAIL_SEGS * M, LANES) for hd in range(k, k + K_GROUP)],
                               axis=1).astype(BF16) for k in range(0, 2 * n_pair, K_GROUP)]
        for j in range(KT):
            acc = None
            for i, k in enumerate(range(0, 2 * n_pair, K_GROUP)):
                part = _dot(lhs[i], _b16(wo[j, k * HALF:(k + K_GROUP) * HALF, :]))
                acc = part if acc is None else acc + part
                for _ in range(2 if state["routed"] else 1):
                    if work and (len(work) > 1 or direct) and next(work[0], "done") == "done":
                        work.pop(0)
            cols = pl.ds(j * LANES, LANES)
            res = base[ss, 0:M, cols] + acc.reshape(TAIL_SEGS, M, LANES)
            if direct:
                xraw[ss, 0:M, cols] = res.astype(BF16)
            else:
                base[ss, 0:M, cols] = res
        if direct:
            out_head(c).start()
    assert not work
    out_rest().wait()
    for c in range(n_chunk):
        out_head(c).wait()


@functools.partial(jax.jit, static_argnames=["A_seg_len"])
def pallas_parallel_sum__memory_aug_recurrent_mem_tr__moe_arch_mod__prompt_kernel(
    A_x, A_mem0, A_Wq, A_Wk, A_Wv, A_Wo, A_seg_len, B_x, B_w_r, B_w_gate, B_w_up, B_w_down,
):
    del B_x
    B, S, D = A_x.shape
    _, H, E = A_Wq.shape
    M = A_mem0.shape[1]
    F = B_w_gate.shape[1]
    seg = A_seg_len
    n_seg = S // seg
    n_pair = H // 2
    KT, FT = D // LANES, F // LANES
    R = 2 * (seg + M)
    assert (B, M, seg, H, E) == (1, 8, 32, 32, LANES) and n_seg * seg == S
    hbm = pl.BlockSpec(memory_space=pl.ANY)
    out = pl.pallas_call(
        _kernel,
        out_shape=jax.ShapeDtypeStruct((n_seg, seg, D), A_x.dtype),
        in_specs=[hbm] * 10,
        out_specs=hbm,
        scratch_shapes=[
            pltpu.VMEM((n_seg, seg, D), BF16),
            pltpu.VMEM((n_seg, seg, D), BF16),
            pltpu.VMEM((KT, n_seg * M // 2, LANES), U32),
            pltpu.VMEM((n_seg, seg, D), F32),
            pltpu.VMEM((RAW_SLOTS, 3, D, LANES), U32),
            pltpu.VMEM((n_pair, 6, D // 2, LANES), U32),
            pltpu.VMEM((KT, H * E // 2, LANES), U32),
            pltpu.VMEM((n_pair, 3, n_seg, M, LANES), U32),
            pltpu.VMEM((H, n_seg, M, LANES), F32),
            pltpu.VMEM((FT, D // 2, LANES), U32),
            pltpu.VMEM((FT, D // 2, LANES), U32),
            pltpu.VMEM((KT, F // 2, LANES), U32),
            pltpu.VMEM((R, R), F32),
            pltpu.VMEM((B, M, D), BF16),
            pltpu.VMEM((D,), BF16),
            pltpu.SemaphoreType.DMA((3,)),
            pltpu.SemaphoreType.DMA((X_CHUNKS,)),
            pltpu.SemaphoreType.DMA((1,)),
            pltpu.SemaphoreType.DMA((RAW_SLOTS, 3)),
            pltpu.SemaphoreType.DMA((1,)),
            pltpu.SemaphoreType.DMA((3,)),
            pltpu.SemaphoreType.DMA((n_seg // TAIL_SEGS + 1,)),
        ],
        compiler_params=pltpu.CompilerParams(vmem_limit_bytes=120 * 1024 * 1024),
    )(A_x.reshape(n_seg, seg, D), A_mem0, A_Wq, A_Wk, A_Wv, A_Wo.reshape(H * E, D),
      B_w_r, B_w_gate, B_w_up, B_w_down)
    return out.reshape(B, S, D)
```

```python
import functools

import jax
import jax.numpy as jnp
import numpy as np
from jax import lax
import jax.experimental.pallas as pl
import jax.experimental.pallas.tpu as pltpu

F32 = jnp.float32
BF16 = jnp.bfloat16
U32 = jnp.uint32
LANES = 128
MASKED = -1000000000.0

X_CHUNKS = 4
PAIRS_PER_ITER = 2
RAW_SLOTS = 2 * PAIRS_PER_ITER
TAIL_SEGS = 8
K_GROUP = 4

STEP_ORDERS = (
    "p0-2 n p3-7 q0-3 p8 q4-7 p9 v0-3 o0 p10-11 o1 p12 o2-3 q8-11 p13 v4-7 p14-15 v8-11 o4-5 "
    "q12-15 o6-9 v12-15 o10-11 o12-15",
    "p0-2 n p3-7 q0-3 p8 q4-7 p9 v0-3 o0 p10-11 o1-2 p12 q8-11 p13 v4-7 p14 o3-5 p15 v8-11 "
    "q12-15 o6-7 o8-10 v12-15 o11 o12 o13 o14-15",
    "p0-2 n p3-5 q0-3 p6-8 q4-7 p9 v0-3 o0 p10-11 o1 p12 q8-11 p13 v4-7 p14 o2-3 p15 v8-11 o4-5 "
    "q12-15 o6-7 v12-15 o8-9 o11 o10 o12-13 o14-15",
)


def _rnd(v):
    return v.astype(BF16).astype(F32)


def _b16(u):
    return pltpu.bitcast(u, BF16)


def _dot(a, b):
    return lax.dot_general(a, b, (((1,), (0,)), ((), ())), preferred_element_type=F32)


def _layernorm(x):
    mean = jnp.mean(x, axis=-1, keepdims=True)
    xc = x - mean
    var = jnp.mean(xc * xc, axis=-1, keepdims=True)
    sd = _rnd(jnp.sqrt(_rnd(_rnd(var) + np.float32(np.asarray(1e-5, BF16)))))
    return _rnd(_rnd(x - _rnd(mean)) / sd)


def _kernel(x_hbm, mem0_hbm, wq_hbm, wk_hbm, wv_hbm, wo_hbm, wr_hbm, wg_hbm, wu_hbm, wd_hbm,
            out_hbm,
            xraw, xn, xa, base, raw, wqkv, wo, sq, so, wg, wu, wd, fill_ref, mem0_ref, wr_ref,
            sem_small, sem_x0, sem_x1, sem_raw, sem_wo, sem_ffn, sem_out):
    n_seg, seg, D = xraw.shape
    M = mem0_ref.shape[1]
    n_pair = wqkv.shape[0]
    KT = D // LANES
    FT = wg.shape[0]
    HALF = LANES // 2
    R = 2 * (seg + M)
    n_r = n_seg * (seg // M) // LANES
    n_chunk = n_seg // TAIL_SEGS
    scale = float(LANES) ** -0.5

    qkv32 = [w.bitcast(U32) for w in (wq_hbm, wk_hbm, wv_hbm)]
    wo32, wg32, wu32, wd32 = (w.bitcast(U32) for w in (wo_hbm, wg_hbm, wu_hbm, wd_hbm))

    def raw_copy(g, slot, c):
        return pltpu.make_async_copy(qkv32[c].at[:, g, :], raw.at[slot, c], sem_raw.at[slot, c])

    def start_pair(g, slot):
        for c in range(3):
            raw_copy(g, slot, c).start()

    def wait_pair(g, slot):
        for c in range(3):
            raw_copy(g, slot, c).wait()

    def x0_copy(i):
        ss = pl.ds(i * (n_seg // X_CHUNKS), n_seg // X_CHUNKS)
        return pltpu.make_async_copy(x_hbm.at[ss, pl.ds(0, M), :], xraw.at[ss, pl.ds(0, M), :], sem_x0.at[i])

    def x1_copy():
        ss = pl.ds(1, n_seg - 1)
        return pltpu.make_async_copy(
            x_hbm.at[ss, pl.ds(M, seg - M), :], xraw.at[ss, pl.ds(M, seg - M), :], sem_x1.at[0])

    def wo_copy(j):
        return pltpu.make_async_copy(
            wo32.at[:, pl.ds(pl.multiple_of(j * LANES, LANES), LANES)], wo.at[j], sem_wo.at[0])

    def ffn_copies():
        cps = []
        for i, (src, dst) in enumerate(((wg32, wg), (wu32, wu), (wd32, wd))):
            for j in range(dst.shape[0]):
                cps.append(pltpu.make_async_copy(src.at[:, pl.ds(j * LANES, LANES)], dst.at[j], sem_ffn.at[i]))
        return cps

    def small_copies():
        return (pltpu.make_async_copy(wr_hbm, wr_ref, sem_small.at[0]),
                pltpu.make_async_copy(mem0_hbm, mem0_ref, sem_small.at[1]),
                pltpu.make_async_copy(x_hbm.at[0, pl.ds(M, seg - M), :], xraw.at[0, pl.ds(M, seg - M), :],
                                      sem_small.at[2]))

    def out_rest():
        return pltpu.make_async_copy(
            xraw.at[:, pl.ds(M, seg - M), :], out_hbm.at[:, pl.ds(M, seg - M), :], sem_out.at[n_chunk])

    def out_head(c):
        ss = pl.ds(c * TAIL_SEGS, TAIL_SEGS)
        return pltpu.make_async_copy(xraw.at[ss, pl.ds(0, M), :], out_hbm.at[ss, pl.ds(0, M), :], sem_out.at[c])

    for i in range(X_CHUNKS):
        x0_copy(i).start()
    raw_copy(0, 0, 0).start()
    for cp in small_copies():
        cp.start()

    def head_and_pos(i):
        head = jnp.where(i < 2 * seg, i // seg, (i - 2 * seg) // M)
        j = i % seg
        pos = jnp.where(i < 2 * seg, jnp.where(j < M, j, j + M), i % M + M)
        return head, pos

    qh, qp = head_and_pos(lax.broadcasted_iota(jnp.int32, (R, R), 0))
    kh, kp = head_and_pos(lax.broadcasted_iota(jnp.int32, (R, R), 1))
    visible = (qp < M) | (qp >= kp)
    fill_ref[...] = jnp.where(qh == kh, jnp.where(visible, 0.0, MASKED), -jnp.inf).astype(F32)

    for i in range(X_CHUNKS):
        x0_copy(i).wait()
        if i == X_CHUNKS - 1:
            raw_copy(0, 0, 1).start()
            raw_copy(0, 0, 2).start()
        for s in range(i * (n_seg // X_CHUNKS), (i + 1) * (n_seg // X_CHUNKS), 2):
            xs = jnp.concatenate([xraw[s, 0:M, :].astype(F32), xraw[s + 1, 0:M, :].astype(F32)], axis=0)
            y = _layernorm(xs).astype(BF16)
            for k in range(KT):
                xa[k, pl.ds(s * (M // 2), M), :] = pltpu.bitcast(y[:, k * LANES:(k + 1) * LANES], U32)

    def project(g, slot, which):
        lhs = jnp.concatenate([_b16(xa[k]) for k in range(KT)], axis=1)
        for c in which:
            even = raw[slot, c, pl.ds(0, D // 2, stride=2), :]
            odd = raw[slot, c, pl.ds(1, D // 2, stride=2), :]
            wa = (even & np.uint32(0xFFFF)) | (odd << 16)
            wb = (even >> 16) | (odd & np.uint32(0xFFFF0000))
            wqkv[g, 2 * c] = wa
            wqkv[g, 2 * c + 1] = wb
            res = _dot(lhs, jnp.concatenate([_b16(wa), _b16(wb)], axis=1))
            a = res[:, :LANES].reshape(n_seg, M, LANES)
            b = res[:, LANES:].reshape(n_seg, M, LANES)
            sq[g, c] = pltpu.bitcast(jnp.concatenate([a, b], axis=1).astype(BF16), U32)

    raw_copy(0, 0, 0).wait()
    start_pair(1, 1)
    project(0, 0, (0,))
    raw_copy(0, 0, 1).wait()
    raw_copy(0, 0, 2).wait()
    start_pair(2, 2)
    project(0, 0, (1, 2))
    wait_pair(1, 1)
    for cp in small_copies():
        cp.wait()
    start_pair(3, 3)
    project(1, 1, (0, 1, 2))

    w_r = wr_ref[...].astype(F32).reshape(1, D)
    lane = lax.broadcasted_iota(jnp.int32, (M, LANES), 1)

    def normalize(s, scores):
        y = _layernorm(xraw[s].astype(F32))
        xn[s] = y.astype(BF16)
        for u in range(seg // M):
            r = _rnd(jnp.sum(y[u * M:(u + 1) * M] * w_r, axis=-1, keepdims=True))
            grp = s * (seg // M) + u
            scores = tuple(jnp.where(lane + LANES * i == grp, r, a) for i, a in enumerate(scores))
        return scores

    scores = normalize(0, tuple(jnp.zeros((M, LANES), F32) for _ in range(n_r)))
    start_pair(RAW_SLOTS, 0)
    start_pair(RAW_SLOTS + 1, 1)

    def phase_a(i, carry):
        g0 = i * PAIRS_PER_ITER
        slot0 = (i % 2) * PAIRS_PER_ITER
        for u in range(PAIRS_PER_ITER):
            wait_pair(g0 + u, slot0 + u)
        for u in range(PAIRS_PER_ITER):
            project(g0 + u, slot0 + u, (0, 1, 2))

        @pl.when(i + 2 < n_pair // PAIRS_PER_ITER)
        def _():
            for u in range(PAIRS_PER_ITER):
                start_pair(g0 + RAW_SLOTS + u, slot0 + u)

        @pl.when(i <= KT // PAIRS_PER_ITER)
        def _():
            for u in range(PAIRS_PER_ITER):
                wo_copy((i - 1) * PAIRS_PER_ITER + u).start()

        @pl.when(i == KT // PAIRS_PER_ITER + 1)
        def _():
            x1_copy().start()

        return carry

    lax.fori_loop(1, n_pair // PAIRS_PER_ITER, phase_a, 0)
    for j in range(KT):
        wo_copy(j).wait()
    x1_copy().wait()
    for cp in ffn_copies():
        cp.start()

    def step(s, carry, u):
        mem, scores = carry

        def rows():
            return jnp.concatenate([mem, xn[s].astype(F32)[M:]], axis=0)

        h = rows().astype(BF16)
        qkv, probs, outs = {}, {}, {}
        acc = None
        for op in STEP_ORDERS[u].split():
            if op == "n":
                base[s] = xraw[s].astype(F32) + xn[s].astype(F32)
                if not isinstance(s, int):
                    nxt = jnp.minimum(s + 1, n_seg - 1)
                    scores = normalize(nxt, scores)
                h = rows().astype(BF16)
                continue
            g0, g1 = (int(t) for t in (op[1:].split("-") * 2)[:2])
            if op[0] == "o":
                lhs = jnp.concatenate([outs.pop(g) for g in range(g0, g1 + 1)], axis=1).astype(BF16)
                res = _dot(lhs, jnp.concatenate(
                    [_b16(wo[j, g0 * LANES:(g1 + 1) * LANES, :]) for j in range(KT)], axis=1))
                acc = res if acc is None else acc + res
                continue
            for g in range(g0, g1 + 1):
                if op[0] == "p":
                    w = jnp.concatenate([_b16(wqkv[g, j]) for j in range(6)], axis=1)
                    if g == 0 and u > 0:
                        hf = rows()
                        res = None
                        for i in range(4):
                            cols = slice(i * D // 4, (i + 1) * D // 4)
                            part = _dot(hf[:, cols].astype(BF16), w[cols])
                            res = part if res is None else res + part
                    else:
                        res = _dot(h, w)
                    qkv[g] = [
                        jnp.concatenate([res[:, (2 * c) * LANES:(2 * c + 1) * LANES],
                                         res[:, (2 * c + 1) * LANES:(2 * c + 2) * LANES],
                                         _b16(sq[g, c, s]).astype(F32)], axis=0).astype(BF16)
                        for c in range(3)]
                elif op[0] == "q":
                    q, k, v = qkv.pop(g)
                    sc = lax.dot_general(q, k, (((1,), (1,)), ((), ())), preferred_element_type=F32) * scale
                    fill = fill_ref[...]
                    sc = jnp.where(fill == 0.0, sc, fill)
                    e = jnp.exp(sc - jnp.max(sc, axis=-1, keepdims=True))
                    total = jnp.sum(e, axis=-1, keepdims=True)
                    inv = pltpu.reciprocal(total, approx=True)
                    inv = inv * (2.0 - total * inv)
                    probs[g] = (e.astype(BF16), inv, v)
                else:
                    e, inv, v = probs.pop(g)
                    o = _dot(e, v) * inv
                    so[2 * g, s] = o[2 * seg:2 * seg + M]
                    so[2 * g + 1, s] = o[2 * seg + M:]
                    outs[g] = jnp.concatenate([o[:seg], o[seg:2 * seg]], axis=1)
        base[s, M:seg, :] = base[s, M:seg, :] + acc[M:]
        return acc[:M], scores

    unroll = len(STEP_ORDERS)

    def steps(i, carry):
        for u in range(unroll):
            carry = step(i * unroll + u, carry, u)
        return carry

    n_iter = (n_seg - 1) // unroll
    assert n_iter * unroll == n_seg - 1
    carry = lax.fori_loop(0, n_iter, steps, (mem0_ref[0].astype(F32), scores))

    for cp in ffn_copies():
        cp.wait()
    _, scores = step(n_seg - 1, carry, 0)

    def routed_ffn():
        tok = [lax.broadcasted_iota(jnp.int32, (M, LANES), 0) + M * (lane + LANES * i) for i in range(n_r)]
        keys = [jnp.where(a != a, -jnp.inf, a) for a in scores]

        def pick(cand):
            best = jnp.max(functools.reduce(jnp.maximum, [jnp.where(c, k, -jnp.inf) for k, c in zip(keys, cand)]))
            return jnp.min(functools.reduce(jnp.minimum, [
                jnp.where(c & (k == best), t, n_seg * seg) for k, t, c in zip(keys, tok, cand)]))

        first = pick([t >= 0 for t in tok])
        second = pick([t != first for t in tok])
        row = lax.broadcasted_iota(jnp.int32, (seg, D), 0)
        slot = lax.broadcasted_iota(jnp.int32, (M, D), 0)
        x_sel = jnp.zeros((M, D), F32)
        for n, i in enumerate((first, second)):
            picked = jnp.sum(jnp.where(row == i % seg, xn[i // seg].astype(F32), 0.0), axis=0, keepdims=True)
            x_sel = jnp.where(slot == n, picked, x_sel)
        weight = jax.nn.sigmoid(_rnd(jnp.sum(x_sel * w_r, axis=-1, keepdims=True)))
        for _ in range(16):
            yield

        hidden = []
        zero = jnp.where(slot[:, :K_GROUP * LANES] < first - n_seg * seg, 1.0, 0.0)
        for j in range(FT):
            gu = zero[:, :2 * LANES]
            for k in range(0, KT, 2):
                tiles = slice(k * HALF, (k + 2) * HALF)
                part = _dot(x_sel[:, k * LANES:(k + 2) * LANES],
                            jnp.concatenate([_b16(wg[j, tiles, :]), _b16(wu[j, tiles, :])], axis=1))
                gu = gu + part
                yield
            gate, up = gu[:, :LANES], gu[:, LANES:]
            hidden.append(_rnd(gate * jax.nn.sigmoid(gate) * up))
        ys = []
        for j0 in range(0, KT, K_GROUP):
            acc = zero
            for k in range(FT):
                part = _dot(hidden[k], jnp.concatenate(
                    [_b16(wd[j, k * HALF:(k + 1) * HALF, :]) for j in range(j0, j0 + K_GROUP)], axis=1))
                acc = part if acc is None else acc + part
                yield
            ys.append(acc)
        y = jnp.concatenate(ys, axis=1) * weight
        for n, i in enumerate((first, second)):
            base[i // seg] = base[i // seg] + jnp.where(row == i % seg, y[n:n + 1], 0.0)

    state = {"routed": False, "early": 0}

    def side_work():
        yield from routed_ffn()
        state["routed"] = True
        for s in range(n_seg):
            xraw[pl.ds(s, 1), M:seg, :] = base[pl.ds(s, 1), M:seg, :].astype(BF16)
            yield
        out_rest().start()

    def early_heads():
        for c in range(state["early"]):
            for s in range(c * TAIL_SEGS, (c + 1) * TAIL_SEGS, 2):
                xraw[pl.ds(s, 2), 0:M, :] = base[pl.ds(s, 2), 0:M, :].astype(BF16)
                yield
            out_head(c).start()

    work = [side_work(), early_heads()]
    for c in range(n_chunk):
        ss = pl.ds(c * TAIL_SEGS, TAIL_SEGS)
        direct = state["routed"]
        if not direct:
            state["early"] = c + 1
        lhs = [jnp.concatenate([so[hd, ss].reshape(TAIL_SEGS * M, LANES) for hd in range(k, k + K_GROUP)],
                               axis=1).astype(BF16) for k in range(0, 2 * n_pair, K_GROUP)]
        for j in range(KT):
            cols = pl.ds(j * LANES, LANES)
            acc = base[ss, 0:M, cols].reshape(TAIL_SEGS * M, LANES)
            for i, k in enumerate(range(0, 2 * n_pair, K_GROUP)):
                acc = acc + _dot(lhs[i], _b16(wo[j, k * HALF:(k + K_GROUP) * HALF, :]))
                for _ in range(2 if state["routed"] else 1):
                    if work and (len(work) > 1 or direct) and next(work[0], "done") == "done":
                        work.pop(0)
            res = acc.reshape(TAIL_SEGS, M, LANES)
            if direct:
                xraw[ss, 0:M, cols] = res.astype(BF16)
            else:
                base[ss, 0:M, cols] = res
        if direct:
            out_head(c).start()
    assert not work
    out_rest().wait()
    for c in range(n_chunk):
        out_head(c).wait()


@functools.partial(jax.jit, static_argnames=["A_seg_len"])
def pallas_parallel_sum__memory_aug_recurrent_mem_tr__moe_arch_mod__prompt_kernel(
    A_x, A_mem0, A_Wq, A_Wk, A_Wv, A_Wo, A_seg_len, B_x, B_w_r, B_w_gate, B_w_up, B_w_down,
):
    del B_x
    B, S, D = A_x.shape
    _, H, E = A_Wq.shape
    M = A_mem0.shape[1]
    F = B_w_gate.shape[1]
    seg = A_seg_len
    n_seg = S // seg
    n_pair = H // 2
    KT, FT = D // LANES, F // LANES
    R = 2 * (seg + M)
    assert (B, M, seg, H, E) == (1, 8, 32, 32, LANES) and n_seg * seg == S
    hbm = pl.BlockSpec(memory_space=pl.ANY)
    out = pl.pallas_call(
        _kernel,
        out_shape=jax.ShapeDtypeStruct((n_seg, seg, D), A_x.dtype),
        in_specs=[hbm] * 10,
        out_specs=hbm,
        scratch_shapes=[
            pltpu.VMEM((n_seg, seg, D), BF16),
            pltpu.VMEM((n_seg, seg, D), BF16),
            pltpu.VMEM((KT, n_seg * M // 2, LANES), U32),
            pltpu.VMEM((n_seg, seg, D), F32),
            pltpu.VMEM((RAW_SLOTS, 3, D, LANES), U32),
            pltpu.VMEM((n_pair, 6, D // 2, LANES), U32),
            pltpu.VMEM((KT, H * E // 2, LANES), U32),
            pltpu.VMEM((n_pair, 3, n_seg, M, LANES), U32),
            pltpu.VMEM((H, n_seg, M, LANES), F32),
            pltpu.VMEM((FT, D // 2, LANES), U32),
            pltpu.VMEM((FT, D // 2, LANES), U32),
            pltpu.VMEM((KT, F // 2, LANES), U32),
            pltpu.VMEM((R, R), F32),
            pltpu.VMEM((B, M, D), BF16),
            pltpu.VMEM((D,), BF16),
            pltpu.SemaphoreType.DMA((3,)),
            pltpu.SemaphoreType.DMA((X_CHUNKS,)),
            pltpu.SemaphoreType.DMA((1,)),
            pltpu.SemaphoreType.DMA((RAW_SLOTS, 3)),
            pltpu.SemaphoreType.DMA((1,)),
            pltpu.SemaphoreType.DMA((3,)),
            pltpu.SemaphoreType.DMA((n_seg // TAIL_SEGS + 1,)),
        ],
        compiler_params=pltpu.CompilerParams(vmem_limit_bytes=120 * 1024 * 1024),
    )(A_x.reshape(n_seg, seg, D), A_mem0, A_Wq, A_Wk, A_Wv, A_Wo.reshape(H * E, D),
      B_w_r, B_w_gate, B_w_up, B_w_down)
    return out.reshape(B, S, D)
```

```python
import functools

import jax
import jax.numpy as jnp
import numpy as np
from jax import lax
import jax.experimental.pallas as pl
import jax.experimental.pallas.tpu as pltpu

F32 = jnp.float32
BF16 = jnp.bfloat16
U32 = jnp.uint32
LANES = 128
MASKED = -1000000000.0

X_CHUNKS = 4
PAIRS_PER_ITER = 2
RAW_SLOTS = 2 * PAIRS_PER_ITER
TAIL_SEGS = 8
K_GROUP = 4

STEP_ORDERS = (
    "p0-2 n p3-7 q0-3 p8 q4-7 p9 v0-3 o0 p10-11 o1 p12 o2-3 q8-11 p13 v4-7 p14-15 v8-11 o4-5 "
    "q12-15 o6-9 v12-15 o10-11 o12-15",
    "p0-2 n p3-7 q0-3 p8 q4-7 p9 v0-3 o0 p10-11 o1-2 p12 q8-11 p13 v4-7 p14 o3-5 p15 v8-11 "
    "q12-15 o6-7 o8-10 v12-15 o11 o12 o13 o14-15",
    "p0-2 n p3-5 q0-3 p6-8 q4-7 p9 v0-3 o0 p10-11 o1 p12 q8-11 p13 v4-7 p14 o2-3 p15 v8-11 o4-5 "
    "q12-15 o6-7 v12-15 o8-9 o11 o10 o12-13 o14-15",
)


def _rnd(v):
    return v.astype(BF16).astype(F32)


def _b16(u):
    return pltpu.bitcast(u, BF16)


def _dot(a, b):
    return lax.dot_general(a, b, (((1,), (0,)), ((), ())), preferred_element_type=F32)


def _layernorm(x):
    mean = jnp.mean(x, axis=-1, keepdims=True)
    xc = x - mean
    var = jnp.mean(xc * xc, axis=-1, keepdims=True)
    sd = _rnd(jnp.sqrt(_rnd(_rnd(var) + np.float32(np.asarray(1e-5, BF16)))))
    return _rnd(_rnd(x - _rnd(mean)) / sd)


def _kernel(x_hbm, mem0_hbm, wq_hbm, wk_hbm, wv_hbm, wo_hbm, wr_hbm, wg_hbm, wu_hbm, wd_hbm,
            out_hbm,
            xraw, xn, xa, base, raw, wqkv, wo, sq, so, wg, wu, wd, fill_ref, mem0_ref, wr_ref,
            sem_small, sem_x0, sem_x1, sem_raw, sem_wo, sem_ffn, sem_out):
    n_seg, seg, D = xraw.shape
    M = mem0_ref.shape[1]
    n_pair = wqkv.shape[0]
    KT = D // LANES
    FT = wg.shape[0]
    HALF = LANES // 2
    R = 2 * (seg + M)
    n_r = n_seg * (seg // M) // LANES
    n_chunk = n_seg // TAIL_SEGS
    scale = float(LANES) ** -0.5

    qkv32 = [w.bitcast(U32) for w in (wq_hbm, wk_hbm, wv_hbm)]
    wo32, wg32, wu32, wd32 = (w.bitcast(U32) for w in (wo_hbm, wg_hbm, wu_hbm, wd_hbm))

    def raw_copy(g, slot, c):
        return pltpu.make_async_copy(qkv32[c].at[:, g, :], raw.at[slot, c], sem_raw.at[slot, c])

    def start_pair(g, slot):
        for c in range(3):
            raw_copy(g, slot, c).start()

    def wait_pair(g, slot):
        for c in range(3):
            raw_copy(g, slot, c).wait()

    def x0_copy(i):
        ss = pl.ds(i * (n_seg // X_CHUNKS), n_seg // X_CHUNKS)
        return pltpu.make_async_copy(x_hbm.at[ss, pl.ds(0, M), :], xraw.at[ss, pl.ds(0, M), :], sem_x0.at[i])

    def x1_copy():
        ss = pl.ds(1, n_seg - 1)
        return pltpu.make_async_copy(
            x_hbm.at[ss, pl.ds(M, seg - M), :], xraw.at[ss, pl.ds(M, seg - M), :], sem_x1.at[0])

    def wo_copy(j):
        return pltpu.make_async_copy(
            wo32.at[:, pl.ds(pl.multiple_of(j * LANES, LANES), LANES)], wo.at[j], sem_wo.at[0])

    def ffn_copies():
        cps = []
        for i, (src, dst) in enumerate(((wg32, wg), (wu32, wu), (wd32, wd))):
            for j in range(dst.shape[0]):
                cps.append(pltpu.make_async_copy(src.at[:, pl.ds(j * LANES, LANES)], dst.at[j], sem_ffn.at[i]))
        return cps

    def small_copies():
        return (pltpu.make_async_copy(wr_hbm, wr_ref, sem_small.at[0]),
                pltpu.make_async_copy(mem0_hbm, mem0_ref, sem_small.at[1]),
                pltpu.make_async_copy(x_hbm.at[0, pl.ds(M, seg - M), :], xraw.at[0, pl.ds(M, seg - M), :],
                                      sem_small.at[2]))

    def out_rest():
        return pltpu.make_async_copy(
            xraw.at[:, pl.ds(M, seg - M), :], out_hbm.at[:, pl.ds(M, seg - M), :], sem_out.at[n_chunk])

    def out_head(c):
        ss = pl.ds(c * TAIL_SEGS, TAIL_SEGS)
        return pltpu.make_async_copy(xraw.at[ss, pl.ds(0, M), :], out_hbm.at[ss, pl.ds(0, M), :], sem_out.at[c])

    for i in range(X_CHUNKS):
        x0_copy(i).start()
    raw_copy(0, 0, 0).start()
    for cp in small_copies():
        cp.start()

    def head_and_pos(i):
        head = jnp.where(i < 2 * seg, i // seg, (i - 2 * seg) // M)
        j = i % seg
        pos = jnp.where(i < 2 * seg, jnp.where(j < M, j, j + M), i % M + M)
        return head, pos

    qh, qp = head_and_pos(lax.broadcasted_iota(jnp.int32, (R, R), 0))
    kh, kp = head_and_pos(lax.broadcasted_iota(jnp.int32, (R, R), 1))
    visible = (qp < M) | (qp >= kp)
    fill_ref[...] = jnp.where(qh == kh, jnp.where(visible, 0.0, MASKED), -jnp.inf).astype(F32)

    for i in range(X_CHUNKS):
        x0_copy(i).wait()
        if i == X_CHUNKS - 1:
            raw_copy(0, 0, 1).start()
            raw_copy(0, 0, 2).start()
        for s in range(i * (n_seg // X_CHUNKS), (i + 1) * (n_seg // X_CHUNKS), 2):
            xs = jnp.concatenate([xraw[s, 0:M, :].astype(F32), xraw[s + 1, 0:M, :].astype(F32)], axis=0)
            y = _layernorm(xs).astype(BF16)
            for k in range(KT):
                xa[k, pl.ds(s * (M // 2), M), :] = pltpu.bitcast(y[:, k * LANES:(k + 1) * LANES], U32)

    def project(g, slot, which):
        lhs = jnp.concatenate([_b16(xa[k]) for k in range(KT)], axis=1)
        for c in which:
            even = raw[slot, c, pl.ds(0, D // 2, stride=2), :]
            odd = raw[slot, c, pl.ds(1, D // 2, stride=2), :]
            wa = (even & np.uint32(0xFFFF)) | (odd << 16)
            wb = (even >> 16) | (odd & np.uint32(0xFFFF0000))
            wqkv[g, 2 * c] = wa
            wqkv[g, 2 * c + 1] = wb
            res = _dot(lhs, jnp.concatenate([_b16(wa), _b16(wb)], axis=1))
            a = res[:, :LANES].reshape(n_seg, M, LANES)
            b = res[:, LANES:].reshape(n_seg, M, LANES)
            sq[g, c] = pltpu.bitcast(jnp.concatenate([a, b], axis=1).astype(BF16), U32)

    raw_copy(0, 0, 0).wait()
    start_pair(1, 1)
    project(0, 0, (0,))
    raw_copy(0, 0, 1).wait()
    raw_copy(0, 0, 2).wait()
    start_pair(2, 2)
    project(0, 0, (1, 2))
    wait_pair(1, 1)
    for cp in small_copies():
        cp.wait()
    start_pair(3, 3)
    project(1, 1, (0, 1, 2))

    w_r = wr_ref[...].astype(F32).reshape(1, D)
    lane = lax.broadcasted_iota(jnp.int32, (M, LANES), 1)

    def normalize(s, scores):
        y = _layernorm(xraw[s].astype(F32))
        xn[s] = y.astype(BF16)
        for u in range(seg // M):
            r = _rnd(jnp.sum(y[u * M:(u + 1) * M] * w_r, axis=-1, keepdims=True))
            grp = s * (seg // M) + u
            scores = tuple(jnp.where(lane + LANES * i == grp, r, a) for i, a in enumerate(scores))
        return scores

    scores = normalize(0, tuple(jnp.zeros((M, LANES), F32) for _ in range(n_r)))
    start_pair(RAW_SLOTS, 0)
    start_pair(RAW_SLOTS + 1, 1)

    def phase_a(i, carry):
        g0 = i * PAIRS_PER_ITER
        slot0 = (i % 2) * PAIRS_PER_ITER
        for u in range(PAIRS_PER_ITER):
            wait_pair(g0 + u, slot0 + u)
        for u in range(PAIRS_PER_ITER):
            project(g0 + u, slot0 + u, (0, 1, 2))

        @pl.when(i + 2 < n_pair // PAIRS_PER_ITER)
        def _():
            for u in range(PAIRS_PER_ITER):
                start_pair(g0 + RAW_SLOTS + u, slot0 + u)

        @pl.when(i <= KT // PAIRS_PER_ITER)
        def _():
            for u in range(PAIRS_PER_ITER):
                wo_copy((i - 1) * PAIRS_PER_ITER + u).start()

        @pl.when(i == KT // PAIRS_PER_ITER + 1)
        def _():
            x1_copy().start()

        return carry

    lax.fori_loop(1, n_pair // PAIRS_PER_ITER, phase_a, 0)
    for j in range(KT):
        wo_copy(j).wait()
    x1_copy().wait()
    for cp in ffn_copies():
        cp.start()

    def step(s, carry, u):
        mem, scores = carry

        def rows():
            return jnp.concatenate([mem, xn[s].astype(F32)[M:]], axis=0)

        h = rows().astype(BF16)
        qkv, probs, outs = {}, {}, {}
        acc = None
        for op in STEP_ORDERS[u].split():
            if op == "n":
                base[s] = xraw[s].astype(F32) + xn[s].astype(F32)
                if not isinstance(s, int):
                    nxt = jnp.minimum(s + 1, n_seg - 1)
                    scores = normalize(nxt, scores)
                h = rows().astype(BF16)
                continue
            g0, g1 = (int(t) for t in (op[1:].split("-") * 2)[:2])
            if op[0] == "o":
                lhs = jnp.concatenate([outs.pop(g) for g in range(g0, g1 + 1)], axis=1).astype(BF16)
                res = _dot(lhs, jnp.concatenate(
                    [_b16(wo[j, g0 * LANES:(g1 + 1) * LANES, :]) for j in range(KT)], axis=1))
                acc = res if acc is None else acc + res
                continue
            for g in range(g0, g1 + 1):
                if op[0] == "p":
                    w = jnp.concatenate([_b16(wqkv[g, j]) for j in range(6)], axis=1)
                    if g == 0 and u > 0:
                        hf = rows()
                        res = None
                        for i in range(4):
                            cols = slice(i * D // 4, (i + 1) * D // 4)
                            part = _dot(hf[:, cols].astype(BF16), w[cols])
                            res = part if res is None else res + part
                    else:
                        res = _dot(h, w)
                    qkv[g] = [
                        jnp.concatenate([res[:, (2 * c) * LANES:(2 * c + 1) * LANES],
                                         res[:, (2 * c + 1) * LANES:(2 * c + 2) * LANES],
                                         _b16(sq[g, c, s]).astype(F32)], axis=0).astype(BF16)
                        for c in range(3)]
                elif op[0] == "q":
                    q, k, v = qkv.pop(g)
                    sc = lax.dot_general(q, k, (((1,), (1,)), ((), ())), preferred_element_type=F32) * scale
                    fill = fill_ref[...]
                    sc = jnp.where(fill == 0.0, sc, fill)
                    e = jnp.exp(sc - jnp.max(sc, axis=-1, keepdims=True))
                    total = jnp.sum(e, axis=-1, keepdims=True)
                    inv = pltpu.reciprocal(total, approx=True)
                    inv = inv * (2.0 - total * inv)
                    probs[g] = (e.astype(BF16), inv, v)
                else:
                    e, inv, v = probs.pop(g)
                    o = _dot(e, v) * inv
                    so[2 * g, s] = o[2 * seg:2 * seg + M]
                    so[2 * g + 1, s] = o[2 * seg + M:]
                    outs[g] = jnp.concatenate([o[:seg], o[seg:2 * seg]], axis=1)
        base[s, M:seg, :] = base[s, M:seg, :] + acc[M:]
        return acc[:M], scores

    unroll = len(STEP_ORDERS)

    def steps(i, carry):
        for u in range(unroll):
            carry = step(i * unroll + u, carry, u)
        return carry

    n_iter = (n_seg - 1) // unroll
    assert n_iter * unroll == n_seg - 1
    carry = lax.fori_loop(0, n_iter, steps, (mem0_ref[0].astype(F32), scores))

    for cp in ffn_copies():
        cp.wait()
    _, scores = step(n_seg - 1, carry, 0)

    tok = [lax.broadcasted_iota(jnp.int32, (M, LANES), 0) + M * (lane + LANES * i) for i in range(n_r)]
    keys = [jnp.where(a != a, -jnp.inf, a) for a in scores]

    def pick(cand):
        best = jnp.max(functools.reduce(jnp.maximum, [jnp.where(c, k, -jnp.inf) for k, c in zip(keys, cand)]))
        return jnp.min(functools.reduce(jnp.minimum, [
            jnp.where(c & (k == best), t, n_seg * seg) for k, t, c in zip(keys, tok, cand)]))

    first = pick([t >= 0 for t in tok])
    second = pick([t != first for t in tok])
    zero = jnp.where(first < 0, 1.0, 0.0).astype(F32)

    def routed_ffn():
        row = lax.broadcasted_iota(jnp.int32, (seg, D), 0)
        slot = lax.broadcasted_iota(jnp.int32, (M, D), 0)
        x_sel = jnp.zeros((M, D), F32)
        for n, i in enumerate((first, second)):
            picked = jnp.sum(jnp.where(row == i % seg, xn[i // seg].astype(F32), 0.0), axis=0, keepdims=True)
            x_sel = jnp.where(slot == n, picked, x_sel)
        weight = jax.nn.sigmoid(_rnd(jnp.sum(x_sel * w_r, axis=-1, keepdims=True)))
        for _ in range(16):
            yield

        hidden = []
        for j in range(FT):
            gu = jnp.full((M, 2 * LANES), zero)
            for k in range(0, KT, 2):
                tiles = slice(k * HALF, (k + 2) * HALF)
                part = _dot(x_sel[:, k * LANES:(k + 2) * LANES],
                            jnp.concatenate([_b16(wg[j, tiles, :]), _b16(wu[j, tiles, :])], axis=1))
                gu = gu + part
                yield
            gate, up = gu[:, :LANES], gu[:, LANES:]
            hidden.append(_rnd(gate * jax.nn.sigmoid(gate) * up))
        ys = []
        for j0 in range(0, KT, K_GROUP):
            acc = jnp.full((M, K_GROUP * LANES), zero)
            for k in range(FT):
                part = _dot(hidden[k], jnp.concatenate(
                    [_b16(wd[j, k * HALF:(k + 1) * HALF, :]) for j in range(j0, j0 + K_GROUP)], axis=1))
                acc = acc + part
                yield
            ys.append(acc)
        y = jnp.concatenate(ys, axis=1) * weight
        for n, i in enumerate((first, second)):
            base[i // seg] = base[i // seg] + jnp.where(row == i % seg, y[n:n + 1], 0.0)

    state = {"routed": False, "early": 0}

    def side_work():
        yield from routed_ffn()
        state["routed"] = True
        for s in range(n_seg):
            xraw[pl.ds(s, 1), M:seg, :] = base[pl.ds(s, 1), M:seg, :].astype(BF16)
            yield
        out_rest().start()

    def early_heads():
        for c in range(state["early"]):
            for s in range(c * TAIL_SEGS, (c + 1) * TAIL_SEGS, 2):
                xraw[pl.ds(s, 2), 0:M, :] = base[pl.ds(s, 2), 0:M, :].astype(BF16)
                yield
            out_head(c).start()

    work = [side_work(), early_heads()]
    for c in range(n_chunk):
        ss = pl.ds(c * TAIL_SEGS, TAIL_SEGS)
        direct = state["routed"]
        if not direct:
            state["early"] = c + 1
        lhs = [jnp.concatenate([so[hd, ss].reshape(TAIL_SEGS * M, LANES) for hd in range(k, k + K_GROUP)],
                               axis=1).astype(BF16) for k in range(0, 2 * n_pair, K_GROUP)]
        for j in range(KT):
            acc = jnp.full((TAIL_SEGS * M, LANES), zero)
            for i, k in enumerate(range(0, 2 * n_pair, K_GROUP)):
                acc = acc + _dot(lhs[i], _b16(wo[j, k * HALF:(k + K_GROUP) * HALF, :]))
                for _ in range(2 if state["routed"] else 1):
                    if work and (len(work) > 1 or direct) and next(work[0], "done") == "done":
                        work.pop(0)
            cols = pl.ds(j * LANES, LANES)
            res = base[ss, 0:M, cols] + acc.reshape(TAIL_SEGS, M, LANES)
            if direct:
                xraw[ss, 0:M, cols] = res.astype(BF16)
            else:
                base[ss, 0:M, cols] = res
        if direct:
            out_head(c).start()
    assert not work
    out_rest().wait()
    for c in range(n_chunk):
        out_head(c).wait()


@functools.partial(jax.jit, static_argnames=["A_seg_len"])
def pallas_parallel_sum__memory_aug_recurrent_mem_tr__moe_arch_mod__prompt_kernel(
    A_x, A_mem0, A_Wq, A_Wk, A_Wv, A_Wo, A_seg_len, B_x, B_w_r, B_w_gate, B_w_up, B_w_down,
):
    del B_x
    B, S, D = A_x.shape
    _, H, E = A_Wq.shape
    M = A_mem0.shape[1]
    F = B_w_gate.shape[1]
    seg = A_seg_len
    n_seg = S // seg
    n_pair = H // 2
    KT, FT = D // LANES, F // LANES
    R = 2 * (seg + M)
    assert (B, M, seg, H, E) == (1, 8, 32, 32, LANES) and n_seg * seg == S
    hbm = pl.BlockSpec(memory_space=pl.ANY)
    out = pl.pallas_call(
        _kernel,
        out_shape=jax.ShapeDtypeStruct((n_seg, seg, D), A_x.dtype),
        in_specs=[hbm] * 10,
        out_specs=hbm,
        scratch_shapes=[
            pltpu.VMEM((n_seg, seg, D), BF16),
            pltpu.VMEM((n_seg, seg, D), BF16),
            pltpu.VMEM((KT, n_seg * M // 2, LANES), U32),
            pltpu.VMEM((n_seg, seg, D), F32),
            pltpu.VMEM((RAW_SLOTS, 3, D, LANES), U32),
            pltpu.VMEM((n_pair, 6, D // 2, LANES), U32),
            pltpu.VMEM((KT, H * E // 2, LANES), U32),
            pltpu.VMEM((n_pair, 3, n_seg, M, LANES), U32),
            pltpu.VMEM((H, n_seg, M, LANES), F32),
            pltpu.VMEM((FT, D // 2, LANES), U32),
            pltpu.VMEM((FT, D // 2, LANES), U32),
            pltpu.VMEM((KT, F // 2, LANES), U32),
            pltpu.VMEM((R, R), F32),
            pltpu.VMEM((B, M, D), BF16),
            pltpu.VMEM((D,), BF16),
            pltpu.SemaphoreType.DMA((3,)),
            pltpu.SemaphoreType.DMA((X_CHUNKS,)),
            pltpu.SemaphoreType.DMA((1,)),
            pltpu.SemaphoreType.DMA((RAW_SLOTS, 3)),
            pltpu.SemaphoreType.DMA((1,)),
            pltpu.SemaphoreType.DMA((3,)),
            pltpu.SemaphoreType.DMA((n_seg // TAIL_SEGS + 1,)),
        ],
        compiler_params=pltpu.CompilerParams(vmem_limit_bytes=120 * 1024 * 1024),
    )(A_x.reshape(n_seg, seg, D), A_mem0, A_Wq, A_Wk, A_Wv, A_Wo.reshape(H * E, D),
      B_w_r, B_w_gate, B_w_up, B_w_down)
    return out.reshape(B, S, D)
```
